```python
import jax
import jax.numpy as jnp

def _softmax(x, axis=-1):
    return jax.nn.softmax(x, axis=axis)

def _gelu(x):
    return jax.nn.gelu(x, approximate=True)

def _silu(x):
    return jax.nn.silu(x)

def _sigmoid(x):
    return jax.nn.sigmoid(x)

def _layernorm(x, axis=-1, eps=1e-05):
    m = jnp.mean(x, axis=axis, keepdims=True)
    v = jnp.var(x, axis=axis, keepdims=True)
    return (x - m) / jnp.sqrt(v + eps)

def _scatter_add(tgt, idx, src, axis=0):
    return tgt.at[idx].add(src)

def _segment_sum(src, seg, n):
    return jax.ops.segment_sum(src, seg, n)

class _Rng:

    def __init__(self, key):
        self._k = key

    def _next(self):
        self._k, sub = jax.random.split(self._k)
        return sub

    def normal(self, shape):
        return jax.random.normal(self._next(), shape, dtype=jnp.bfloat16)

    def randint(self, lo, hi, shape):
        return jax.random.randint(self._next(), shape, lo, hi, dtype=jnp.int32)

    def uniform(self, shape, lo=0.0, hi=1.0):
        return jax.random.uniform(self._next(), shape, jnp.bfloat16, lo, hi)

    def permutation(self, n):
        return jax.random.permutation(self._next(), n)
kernel_name = 'adaLN_cond__sliding_block_cached__dense_activation_mish__decode'

def setup_inputs():
    _rng = _Rng(jax.random.key(int.from_bytes(__import__("os").urandom(4), "little")))
    _w = lambda a: (lambda t: t.astype(jnp.bfloat16) if jnp.issubdtype(t.dtype, jnp.floating) else t)(jnp.asarray(a))

    def _A_setup():
        B, Sq, D = (1, 1, 640)
        Hq, Hkv, Sk, Dh = (32, 32, 32768, 192)
        assert Hq % Hkv == 0, (Hq, Hkv)
        return {'x': _w((lambda *s: _rng.normal(s) * 0.05)(B, Sq, D)), 'k_cache': _w((lambda *s: _rng.normal(s) * 0.05)(B, Hkv, Sk, Dh)), 'v_cache': _w((lambda *s: _rng.normal(s) * 0.05)(B, Hkv, Sk, Dh)), 'wq': _w((lambda *s: _rng.normal(s) * 0.05)(D, Hq * Dh) * D ** (-0.5)), 'wo': _w((lambda *s: _rng.normal(s) * 0.05)(Hq * Dh, D) * (Hq * Dh) ** (-0.5))}
    _A_in = _A_setup()

    def _B_setup():
        B, S, D, F = (1, 1, 640, 1536)
        return {'x': _w((lambda *s: _rng.normal(s) * 0.05)(B, S, D)), 'w1': _w((lambda *s: _rng.normal(s) * 0.05)(D, F) * D ** (-0.5)), 'b1': _w((lambda *s: _rng.normal(s) * 0.05)(F)), 'w2': _w((lambda *s: _rng.normal(s) * 0.05)(F, D) * F ** (-0.5))}
    _B_in = _B_setup()
    return {'A_x': _A_in['x'], 'A_k_cache': _A_in['k_cache'], 'A_v_cache': _A_in['v_cache'], 'A_wq': _A_in['wq'], 'A_wo': _A_in['wo'], 'B_x': _B_in['x'], 'B_w1': _B_in['w1'], 'B_b1': _B_in['b1'], 'B_w2': _B_in['w2'], 'c': _w((lambda *s: _rng.normal(s) * 0.05)(1, 640)), 'w_mod': _w((lambda *s: _rng.normal(s) * 0.05)(640, 6 * 640) * 640 ** (-0.5))}

def reference(A_x, A_k_cache, A_v_cache, A_wq, A_wo, B_x, B_w1, B_b1, B_w2, c, w_mod):

    def _A_ref(x, k_cache, v_cache, wq, wo):
        B, Sq, D = x.shape
        Hq, Dh = (32, 192)
        Hkv, Sk = (k_cache.shape[1], k_cache.shape[2])
        W = min(4096, max(256, Sk // 4))
        rep = Hq // Hkv
        q = (lambda x, *d: x.transpose(*d))((x @ wq).reshape(B, Sq, Hq, Dh), 0, 2, 1, 3)
        k = jnp.repeat(k_cache[:, :, Sk - W:, :], rep, axis=1)
        v = jnp.repeat(v_cache[:, :, Sk - W:, :], rep, axis=1)
        scores = jnp.einsum('bhqd,bhkd->bhqk', q, k) * Dh ** (-0.5)
        p = _softmax(scores, axis=-1)
        o = jnp.einsum('bhqk,bhkd->bhqd', p, v)
        return (lambda x, *d: x.transpose(*d))(o, 0, 2, 1, 3).reshape(B, Sq, Hq * Dh) @ wo

    def _B_ref(x, w1, b1, w2):
        h = jnp.einsum('bsd,df->bsf', x, w1) + b1
        sp = jnp.log1p(jnp.exp(-jnp.abs(h))) + jnp.where(h > 0, h, jnp.zeros_like(h))
        act = h * jnp.tanh(sp)
        return jnp.einsum('bsf,fd->bsd', act, w2)
    x = A_x
    mod = (_silu(c) @ w_mod).reshape(c.shape[0], 6, 1, -1)
    sa, ca, ga, sb, cb, gb = (mod[:, 0].copy(), mod[:, 1].copy(), mod[:, 2].copy(), mod[:, 3].copy(), mod[:, 4].copy(), mod[:, 5].copy())
    h = _layernorm(x, axis=-1) * (1 + ca) + sa
    x = x + ga * _A_ref(h, A_k_cache, A_v_cache, A_wq, A_wo)
    h = _layernorm(x, axis=-1) * (1 + cb) + sb
    x = x + gb * _B_ref(h, B_w1, B_b1, B_w2)
    return x
```

```python
import functools

import jax
import jax.numpy as jnp
from jax import lax
import jax.experimental.pallas as pl
import jax.experimental.pallas.tpu as pltpu

D = 640
H = 32
DH = 192
F = 1536
PAIR = 2 * DH
NPAIR = H // 2
NBUF = 8
WQ_CHUNKS = 4
W2_CHUNKS = (512, 512, 256, 128, 128)
EPS = 1e-5

f32 = jnp.float32
bf16 = jnp.bfloat16


def _layernorm(x):
    m = jnp.mean(x, axis=-1, keepdims=True)
    xc = x - m
    v = jnp.mean(xc * xc, axis=-1, keepdims=True)
    return xc / jnp.sqrt(v + EPS)


def _kernel(x_hbm, c_hbm, b1_hbm, wmod_hbm, wq_hbm, k_hbm, v_hbm, wo_hbm, w1_hbm, w2_hbm,
            out_hbm,
            x_v, c_v, b1_v, wmod_v, wq_v, kv_buf, wo_v, w1_v, w2_v, q_s, o_s, out_v,
            small_sem, wmod_sem, wq_sem, kv_sem, wo_sem, w1_sem, w2_sem, out_sem,
            *, W, SK):
    col0 = SK - W
    wq_cols = (H * DH) // WQ_CHUNKS

    x_cp = pltpu.make_async_copy(x_hbm, x_v, small_sem.at[0])
    c_cp = pltpu.make_async_copy(c_hbm, c_v, small_sem.at[1])
    b1_cp = pltpu.make_async_copy(b1_hbm, b1_v, small_sem.at[2])
    wmod_a = pltpu.make_async_copy(wmod_hbm.at[:, pl.ds(0, 2 * D)], wmod_v.at[:, pl.ds(0, 2 * D)], wmod_sem.at[0])
    wmod_b = pltpu.make_async_copy(wmod_hbm.at[:, pl.ds(2 * D, 4 * D)], wmod_v.at[:, pl.ds(2 * D, 4 * D)], wmod_sem.at[1])

    def wq_cp(j):
        return pltpu.make_async_copy(wq_hbm.at[:, pl.ds(j * wq_cols, wq_cols)],
                                     wq_v.at[:, pl.ds(j * wq_cols, wq_cols)], wq_sem.at[j])

    def kv_cp(src, p, slot):
        r0 = p * PAIR
        if not isinstance(p, int):
            r0 = pl.multiple_of(r0, PAIR)
        return pltpu.make_async_copy(src.at[pl.ds(r0, PAIR), pl.ds(col0, W)], kv_buf.at[slot], kv_sem.at[slot])

    wo_cp = pltpu.make_async_copy(wo_hbm, wo_v, wo_sem.at[0])
    w1_cp = pltpu.make_async_copy(w1_hbm, w1_v, w1_sem.at[0])
    w2_offs = [sum(W2_CHUNKS[:j]) for j in range(len(W2_CHUNKS))]

    def w2_cp(j):
        return pltpu.make_async_copy(w2_hbm.at[pl.ds(w2_offs[j], W2_CHUNKS[j]), :],
                                     w2_v.at[pl.ds(w2_offs[j], W2_CHUNKS[j]), :], w2_sem.at[j])

    c_cp.start()
    x_cp.start()
    wmod_a.start()
    for j in range(WQ_CHUNKS):
        wq_cp(j).start()
    for s in range(NBUF):
        kv_cp(k_hbm if s % 2 == 0 else v_hbm, s // 2, s).start()
    b1_cp.start()
    wmod_b.start(priority=1)
    wo_cp.start(priority=1)
    w1_cp.start(priority=1)
    for j in range(len(W2_CHUNKS)):
        w2_cp(j).start(priority=1)

    c_cp.wait()
    x_cp.wait()
    c32 = c_v[...].astype(f32)
    sc = c32 * jax.nn.sigmoid(c32)
    sc8 = jnp.broadcast_to(sc, (8, D)).astype(bf16)
    x32 = x_v[...].astype(f32)
    xn = _layernorm(x32)
    wmod_a.wait()
    mod_a = jnp.dot(sc8, wmod_v[:, 0:2 * D], preferred_element_type=f32)
    h = xn * (1.0 + mod_a[:, D:2 * D]) + mod_a[:, 0:D]
    h8 = h.astype(bf16)

    row = lax.broadcasted_iota(jnp.int32, (8, PAIR), 0)
    lane = lax.broadcasted_iota(jnp.int32, (8, PAIR), 1)
    diag = (row == jnp.where(lane >= DH, 1, 0))
    ppc = NPAIR // WQ_CHUNKS
    for j in range(WQ_CHUNKS):
        wq_cp(j).wait()
        qj = jnp.dot(h8, wq_v[:, j * wq_cols:(j + 1) * wq_cols], preferred_element_type=f32)
        for t in range(ppc):
            q_s[j * ppc + t] = jnp.where(diag, qj[:, t * PAIR:(t + 1) * PAIR], 0.0)

    scale = DH ** -0.5

    def pair_step(p, carry):
        ks = (2 * p) % NBUF
        vs = ks + 1
        kv_cp(k_hbm, p, ks).wait()
        q2 = q_s[p].astype(bf16)
        s = jnp.dot(q2, kv_buf[ks], preferred_element_type=f32) * scale

        @pl.when(p + NBUF // 2 < NPAIR)
        def _():
            kv_cp(k_hbm, p + NBUF // 2, ks).start()

        m = jnp.max(s, axis=-1, keepdims=True)
        e = jnp.exp(s - m)
        l = jnp.sum(e, axis=-1, keepdims=True)
        kv_cp(v_hbm, p, vs).wait()
        o2 = lax.dot_general(e.astype(bf16), kv_buf[vs], (((1,), (1,)), ((), ())),
                             preferred_element_type=f32)

        @pl.when(p + NBUF // 2 < NPAIR)
        def _():
            kv_cp(v_hbm, p + NBUF // 2, vs).start()

        o2 = jnp.where(diag, o2 / l, 0.0)
        o_s[p] = jnp.broadcast_to(jnp.sum(o2, axis=0, keepdims=True), (8, PAIR))
        return carry

    lax.fori_loop(0, NPAIR, pair_step, 0)

    wmod_b.wait()
    mod_b = jnp.dot(sc8, wmod_v[:, 2 * D:6 * D], preferred_element_type=f32)
    ga, sb, cb, gb = (mod_b[:, i * D:(i + 1) * D] for i in range(4))
    wo_cp.wait()
    attn = jnp.zeros((8, D), f32)
    for p in range(NPAIR):
        attn = attn + jnp.dot(o_s[p].astype(bf16), wo_v[p * PAIR:(p + 1) * PAIR, :], preferred_element_type=f32)
    x1 = x32 + ga * attn

    h2 = (_layernorm(x1) * (1.0 + cb) + sb).astype(bf16)
    b1_cp.wait()
    w1_cp.wait()
    b1 = b1_v[...].astype(f32)
    b1row = jnp.concatenate([b1[j:j + 1, :] for j in range(F // 128)], axis=1)
    u = jnp.dot(h2, w1_v[...], preferred_element_type=f32) + b1row
    sp = jnp.log1p(jnp.exp(-jnp.abs(u))) + jnp.maximum(u, 0.0)
    act = (u * jnp.tanh(sp)).astype(bf16)
    y = jnp.zeros((8, D), f32)
    for j in range(len(W2_CHUNKS)):
        w2_cp(j).wait()
        o0, n = w2_offs[j], W2_CHUNKS[j]
        y = y + jnp.dot(act[:, o0:o0 + n], w2_v[o0:o0 + n, :], preferred_element_type=f32)
    res = x1 + gb * y
    out_v[...] = res[0:1, :].astype(bf16)
    out_cp = pltpu.make_async_copy(out_v, out_hbm, out_sem.at[0])
    out_cp.start()
    out_cp.wait()


@jax.jit
def pallas_adaLN_cond__sliding_block_cached__dense_activation_mish__decode_kernel(
    A_x: jax.Array,
    A_k_cache: jax.Array,
    A_v_cache: jax.Array,
    A_wq: jax.Array,
    A_wo: jax.Array,
    B_x: jax.Array,
    B_w1: jax.Array,
    B_b1: jax.Array,
    B_w2: jax.Array,
    c: jax.Array,
    w_mod: jax.Array,
):
    del B_x
    SK = A_k_cache.shape[2]
    W = min(4096, max(256, SK // 4))
    kt = jnp.swapaxes(A_k_cache, 2, 3).reshape(H * DH, SK)
    vt = jnp.swapaxes(A_v_cache, 2, 3).reshape(H * DH, SK)
    x = A_x.reshape(1, D)
    b1 = B_b1.reshape(F // 128, 128)

    any_spec = pl.BlockSpec(memory_space=pl.ANY)
    out = pl.pallas_call(
        functools.partial(_kernel, W=W, SK=SK),
        out_shape=jax.ShapeDtypeStruct((1, D), bf16),
        in_specs=[any_spec] * 10,
        out_specs=any_spec,
        scratch_shapes=[
            pltpu.VMEM((1, D), bf16),
            pltpu.VMEM((1, D), bf16),
            pltpu.VMEM((F // 128, 128), bf16),
            pltpu.VMEM((D, 6 * D), bf16),
            pltpu.VMEM((D, H * DH), bf16),
            pltpu.VMEM((NBUF, PAIR, W), bf16),
            pltpu.VMEM((H * DH, D), bf16),
            pltpu.VMEM((D, F), bf16),
            pltpu.VMEM((F, D), bf16),
            pltpu.VMEM((NPAIR, 8, PAIR), f32),
            pltpu.VMEM((NPAIR, 8, PAIR), f32),
            pltpu.VMEM((1, D), bf16),
            pltpu.SemaphoreType.DMA((3,)),
            pltpu.SemaphoreType.DMA((2,)),
            pltpu.SemaphoreType.DMA((WQ_CHUNKS,)),
            pltpu.SemaphoreType.DMA((NBUF,)),
            pltpu.SemaphoreType.DMA((1,)),
            pltpu.SemaphoreType.DMA((1,)),
            pltpu.SemaphoreType.DMA((len(W2_CHUNKS),)),
            pltpu.SemaphoreType.DMA((1,)),
        ],
        compiler_params=pltpu.CompilerParams(vmem_limit_bytes=100 * 1024 * 1024),
    )(x, c, b1, w_mod, A_wq, kt, vt, A_wo, B_w1, B_w2)
    return out.reshape(1, 1, D)
```

```python
import functools

import jax
import jax.numpy as jnp
from jax import lax
import jax.experimental.pallas as pl
import jax.experimental.pallas.tpu as pltpu

D = 640
H = 32
DH = 192
F = 1536
PAIR = 2 * DH
NPAIR = H // 2
AHEAD = 4
NBUF = 2 * AHEAD
WQ_CHUNKS = 4
EPS = 1e-5

NS = 3
A_ROWS, A_COLS = 40, 2 * D
NA = (D // A_ROWS) * 2
B_ROWS = 80
NB = 5
NSIDE = NA + NB
PRE_EVENTS = 5
SPRIO = 0
W2_MAIN0 = NB * B_ROWS
W2_BOUNDS = [b for b in (W2_MAIN0, 768, 1152, 1408, F) if b >= W2_MAIN0]
NW2 = len(W2_BOUNDS) - 1

f32 = jnp.float32
bf16 = jnp.bfloat16

S_C, S_X, S_B1, S_WMA, S_W1, S_OUT = range(6)
S_WQ = 6
S_W2 = S_WQ + WQ_CHUNKS
S_KV = S_W2 + NW2
S_WO = S_KV + NBUF
S_IN = S_WO + AHEAD
S_SV = S_IN + NS
NSEM = S_SV + NS


def _layernorm(x):
    m = jnp.mean(x, axis=-1, keepdims=True)
    xc = x - m
    v = jnp.mean(xc * xc, axis=-1, keepdims=True)
    return xc / jnp.sqrt(v + EPS)


def _kernel(x_hbm, c_hbm, b1_hbm, wmod_hbm, wq_hbm, k_hbm, v_hbm, wo_hbm, w1_hbm, w2_hbm,
            out_hbm,
            x_v, c_v, b1_v, wmod_v, wq_v, kv_buf, wo_v, w1_v, w2_v, q_s, out_v, sa_s, sb_s, sem,
            *, W, SK):
    col0 = SK - W
    wq_cols = (H * DH) // WQ_CHUNKS

    x_cp = pltpu.make_async_copy(x_hbm, x_v, sem.at[S_X])
    c_cp = pltpu.make_async_copy(c_hbm, c_v, sem.at[S_C])
    b1_cp = pltpu.make_async_copy(b1_hbm, b1_v, sem.at[S_B1])
    wmod_a = pltpu.make_async_copy(wmod_hbm.at[:, pl.ds(0, 2 * D)], wmod_v.at[:, pl.ds(0, 2 * D)], sem.at[S_WMA])

    def wq_cp(j):
        return pltpu.make_async_copy(wq_hbm.at[:, pl.ds(j * wq_cols, wq_cols)],
                                     wq_v.at[:, pl.ds(j * wq_cols, wq_cols)], sem.at[S_WQ + j])

    def rows(p):
        r0 = p * PAIR
        if not isinstance(p, int):
            r0 = pl.multiple_of(r0, PAIR)
        return pl.ds(r0, PAIR)

    def kv_cp(src, p, slot):
        return pltpu.make_async_copy(src.at[rows(p), pl.ds(col0, W)], kv_buf.at[slot], sem.at[S_KV + slot])

    def wo_cp(p, slot):
        return pltpu.make_async_copy(wo_hbm.at[rows(p), :], wo_v.at[slot], sem.at[S_WO + slot])

    w1_cp = pltpu.make_async_copy(w1_hbm, w1_v, sem.at[S_W1])

    def w2_cp(j):
        sl = pl.ds(W2_BOUNDS[j], W2_BOUNDS[j + 1] - W2_BOUNDS[j])
        return pltpu.make_async_copy(w2_hbm.at[sl, :], w2_v.at[sl, :], sem.at[S_W2 + j])

    def mult(v, m):
        return v if isinstance(v, int) else pl.multiple_of(v, m)

    def side_a(j, inbound):
        slot = j % NS
        r = pl.ds(mult((j // 2) * A_ROWS, 8), A_ROWS)
        cs = pl.ds(mult(2 * D + (j % 2) * A_COLS, 128), A_COLS)
        if inbound:
            return pltpu.make_async_copy(wmod_hbm.at[r, cs], sa_s.at[slot], sem.at[S_IN + slot])
        return pltpu.make_async_copy(sa_s.at[slot], wmod_v.at[r, cs], sem.at[S_SV + slot])

    def side_b(j, inbound):
        slot = j % NS
        r = pl.ds(mult((j - NA) * B_ROWS, 8), B_ROWS)
        if inbound:
            return pltpu.make_async_copy(w2_hbm.at[r, :], sb_s.at[slot], sem.at[S_IN + slot])
        return pltpu.make_async_copy(sb_s.at[slot], w2_v.at[r, :], sem.at[S_SV + slot])

    def side_do(j, inbound, op):
        if isinstance(j, int):
            if 0 <= j < NA:
                op(side_a(j, inbound))
            elif NA <= j < NSIDE:
                op(side_b(j, inbound))
            return

        @pl.when(j < NA)
        def _():
            op(side_a(j, inbound))

        if NB:
            @pl.when(jnp.logical_and(j >= NA, j < NSIDE))
            def _():
                op(side_b(j, inbound))

    start = lambda d: d.start(priority=SPRIO)
    wait = lambda d: d.wait()

    def side_event(j):
        side_do(j, True, wait)
        side_do(j, False, start)
        side_do(j - 1, False, wait)
        side_do(j - 1 + NS, True, start)

    wmod_a.start()
    c_cp.start()
    x_cp.start()
    for j in range(NS - 1):
        side_do(j, True, start)
    for j in range(WQ_CHUNKS):
        wq_cp(j).start()
    for p in range(AHEAD):
        kv_cp(k_hbm, p, 2 * p).start()
        wo_cp(p, p).start()
        kv_cp(v_hbm, p, 2 * p + 1).start()
    b1_cp.start(priority=1)
    w1_cp.start(priority=1)
    for j in range(NW2):
        w2_cp(j).start(priority=1)

    c_cp.wait()
    x_cp.wait()
    c32 = c_v[...].astype(f32)
    sc = c32 * jax.nn.sigmoid(c32)
    sc8 = jnp.broadcast_to(sc, (8, D)).astype(bf16)
    x32 = x_v[...].astype(f32)
    xn = _layernorm(x32)
    ev = 0
    wmod_a.wait()
    if ev < PRE_EVENTS:
        side_event(ev)
        ev += 1
    mod_a = jnp.dot(sc8, wmod_v[:, 0:2 * D], preferred_element_type=f32)
    h = xn * (1.0 + mod_a[:, D:2 * D]) + mod_a[:, 0:D]
    h8 = h.astype(bf16)

    row = lax.broadcasted_iota(jnp.int32, (8, PAIR), 0)
    lane = lax.broadcasted_iota(jnp.int32, (8, PAIR), 1)
    diag = (row == jnp.where(lane >= DH, 1, 0))
    ppc = NPAIR // WQ_CHUNKS
    for j in range(WQ_CHUNKS):
        wq_cp(j).wait()
        if j >= 1 and ev < PRE_EVENTS:
            side_event(ev)
            ev += 1
        qj = jnp.dot(h8, wq_v[:, j * wq_cols:(j + 1) * wq_cols], preferred_element_type=f32)
        for t in range(ppc):
            q_s[j * ppc + t] = jnp.where(diag, qj[:, t * PAIR:(t + 1) * PAIR], 0.0)
    while ev < PRE_EVENTS:
        side_event(ev)
        ev += 1

    scale = DH ** -0.5

    def pair_step(p, acc):
        slot = p % AHEAD
        ks = 2 * slot
        vs = ks + 1
        kv_cp(k_hbm, p, ks).wait()
        side_event(PRE_EVENTS + 2 * p)
        q2 = q_s[p].astype(bf16)
        s = jnp.dot(q2, kv_buf[ks], preferred_element_type=f32) * scale

        @pl.when(p + AHEAD < NPAIR)
        def _():
            kv_cp(k_hbm, p + AHEAD, ks).start()

        m = jnp.max(s, axis=-1, keepdims=True)
        e = jnp.exp(s - m)
        l = jnp.sum(e, axis=-1, keepdims=True)
        kv_cp(v_hbm, p, vs).wait()
        side_event(PRE_EVENTS + 2 * p + 1)
        o2 = lax.dot_general(e.astype(bf16), kv_buf[vs], (((1,), (1,)), ((), ())),
                             preferred_element_type=f32)
        o2 = jnp.where(diag, o2 / l, 0.0).astype(bf16)
        wo_cp(p, slot).wait()
        acc = acc + jnp.dot(o2, wo_v[slot], preferred_element_type=f32)

        @pl.when(p + AHEAD < NPAIR)
        def _():
            wo_cp(p + AHEAD, slot).start()
            kv_cp(v_hbm, p + AHEAD, vs).start()

        return acc

    acc = lax.fori_loop(0, NPAIR, pair_step, jnp.zeros((8, D), f32))
    attn = jnp.sum(acc, axis=0, keepdims=True)
    ev = PRE_EVENTS + 2 * NPAIR
    while ev <= NA:
        side_event(ev)
        ev += 1

    mod_b = jnp.dot(sc8, wmod_v[:, 2 * D:6 * D], preferred_element_type=f32)
    ga, sb, cb, gb = (mod_b[:, i * D:(i + 1) * D] for i in range(4))
    x1 = x32 + ga * attn

    h2 = (_layernorm(x1) * (1.0 + cb) + sb).astype(bf16)
    b1_cp.wait()
    b1 = b1_v[...].astype(f32)
    b1row = jnp.concatenate([b1[j:j + 1, :] for j in range(F // 128)], axis=1)
    w1_cp.wait()
    if ev <= NSIDE:
        side_event(ev)
        ev += 1
    u = jnp.dot(h2, w1_v[...], preferred_element_type=f32) + b1row
    sp = jnp.log1p(jnp.exp(-jnp.abs(u))) + jnp.maximum(u, 0.0)
    act = (u * jnp.tanh(sp)).astype(bf16)
    y = jnp.zeros((8, D), f32)
    while ev <= NSIDE:
        side_event(ev)
        ev += 1
    for j in range(NW2):
        w2_cp(j).wait()
        o0 = 0 if j == 0 else W2_BOUNDS[j]
        o1 = W2_BOUNDS[j + 1]
        y = y + jnp.dot(act[:, o0:o1], w2_v[o0:o1, :], preferred_element_type=f32)
    res = x1 + gb * y
    out_v[...] = res[0:1, :].astype(bf16)
    out_cp = pltpu.make_async_copy(out_v, out_hbm, sem.at[S_OUT])
    out_cp.start()
    out_cp.wait()


@jax.jit
def pallas_adaLN_cond__sliding_block_cached__dense_activation_mish__decode_kernel(
    A_x: jax.Array,
    A_k_cache: jax.Array,
    A_v_cache: jax.Array,
    A_wq: jax.Array,
    A_wo: jax.Array,
    B_x: jax.Array,
    B_w1: jax.Array,
    B_b1: jax.Array,
    B_w2: jax.Array,
    c: jax.Array,
    w_mod: jax.Array,
):
    del B_x
    SK = A_k_cache.shape[2]
    W = min(4096, max(256, SK // 4))
    kt = jnp.swapaxes(A_k_cache, 2, 3).reshape(H * DH, SK)
    vt = jnp.swapaxes(A_v_cache, 2, 3).reshape(H * DH, SK)
    x = A_x.reshape(1, D)
    b1 = B_b1.reshape(F // 128, 128)

    any_spec = pl.BlockSpec(memory_space=pl.ANY)
    out = pl.pallas_call(
        functools.partial(_kernel, W=W, SK=SK),
        out_shape=jax.ShapeDtypeStruct((1, D), bf16),
        in_specs=[any_spec] * 10,
        out_specs=any_spec,
        scratch_shapes=[
            pltpu.VMEM((1, D), bf16),
            pltpu.VMEM((1, D), bf16),
            pltpu.VMEM((F // 128, 128), bf16),
            pltpu.VMEM((D, 6 * D), bf16),
            pltpu.VMEM((D, H * DH), bf16),
            pltpu.VMEM((NBUF, PAIR, W), bf16),
            pltpu.VMEM((AHEAD, PAIR, D), bf16),
            pltpu.VMEM((D, F), bf16),
            pltpu.VMEM((F, D), bf16),
            pltpu.VMEM((NPAIR, 8, PAIR), f32),
            pltpu.VMEM((1, D), bf16),
            pltpu.SMEM((NS, A_ROWS, A_COLS), bf16),
            pltpu.SMEM((NS, B_ROWS, D), bf16),
            pltpu.SemaphoreType.DMA((NSEM,)),
        ],
        compiler_params=pltpu.CompilerParams(
            vmem_limit_bytes=100 * 1024 * 1024,
            disable_bounds_checks=True,
            disable_semaphore_checks=True,
        ),
    )(x, c, b1, w_mod, A_wq, kt, vt, A_wo, B_w1, B_w2)
    return out.reshape(1, 1, D)
```

```python
import functools

import jax
import jax.numpy as jnp
from jax import lax
import jax.experimental.pallas as pl
import jax.experimental.pallas.tpu as pltpu

D = 640
H = 32
DH = 192
F = 1536
PAIR = 2 * DH
NPAIR = H // 2
AHEAD = 4
NBUF = 2 * AHEAD
KVSPLIT = 2
WQ_CHUNKS = 4
EPS = 1e-5

MG, MR = 10, 64
QG, QR = 8, 80
WO_SLAB = 48
NSLAB = PAIR // WO_SLAB
SLAB_PER = NSLAB // 8
MSLAB = 1
QSLAB = 1
OSLAB = 1

NS = 4
LAG = 2
A_COLS = 2 * D
NA = (D // 8) * 2
B_ROWS = 16
NB = 23
NSIDE = NA + NB
PRE = (3, 3, 3, 3, 3, 5)
R_PAIR = 2482
R_SLAB = 379
R_V = 1241
PHASE = 128
POST = (2, 9)
MODB_AT = 15
W2_MAIN0 = NB * B_ROWS
W2_BOUNDS = [W2_MAIN0] + [b for b in (768, 1152, 1408, F) if b > W2_MAIN0]
NW2 = len(W2_BOUNDS) - 1
SIDE_K = -(-W2_MAIN0 // 128) * 128
SIDE_AFTER = 1

f32 = jnp.float32
bf16 = jnp.bfloat16

S_C, S_X, S_B1, S_WMA, S_W1, S_OUT, S_WO = range(7)
S_WQ = 7
S_W2 = S_WQ + WQ_CHUNKS
S_KV = S_W2 + NW2
S_IN = S_KV + NBUF
S_SV = S_IN + NS
NSEM = S_SV + NS


def _layernorm(x):
    m = jnp.mean(x, axis=-1, keepdims=True)
    xc = x - m
    v = jnp.mean(xc * xc, axis=-1, keepdims=True)
    return xc / jnp.sqrt(v + EPS)


def _kernel(x_hbm, c_hbm, b1_hbm, wmod_hbm, wq_hbm, k_hbm, v_hbm, wo_hbm, w1_hbm, w2_hbm,
            out_hbm,
            x_v, c_v, b1_v, wmod_v, wq_v, kv_buf, wo_v, w1_v, w2_v, q_s, o_s, acc_s, modb_s, out_v, sa_s, sb_s, sem,
            *, W, SK):
    col0 = SK - W
    wq_cols = (H * DH) // WQ_CHUNKS
    wc = W // KVSPLIT

    def mult(v, m):
        return v if isinstance(v, int) else pl.multiple_of(v, m)

    x_cp = pltpu.make_async_copy(x_hbm, x_v, sem.at[S_X])
    c_cp = pltpu.make_async_copy(c_hbm, c_v, sem.at[S_C])
    b1_cp = pltpu.make_async_copy(b1_hbm, b1_v, sem.at[S_B1])

    def wma_cp(i, n):
        idx = (slice(None), pl.ds(8 * i, n), pl.ds(0, 2 * D))
        return pltpu.make_async_copy(wmod_hbm.at[idx], wmod_v.at[idx], sem.at[S_WMA])

    def wq_cp(j, i, n):
        idx = (slice(None), pl.ds(8 * i, n), pl.ds(j * wq_cols, wq_cols))
        return pltpu.make_async_copy(wq_hbm.at[idx], wq_v.at[idx], sem.at[S_WQ + j])

    def kv_cps(src, p, slot):
        rows = pl.ds(mult(p * PAIR, PAIR), PAIR)
        return [pltpu.make_async_copy(src.at[rows, pl.ds(col0 + t * wc, wc)],
                                      kv_buf.at[slot, t], sem.at[S_KV + slot])
                for t in range(KVSPLIT)]

    def kv_start(src, p, slot):
        for d in kv_cps(src, p, slot):
            d.start()

    def kv_wait(src, p, slot):
        for d in kv_cps(src, p, slot):
            d.wait()

    def wo_start(p):
        if OSLAB:
            for t in range(SLAB_PER):
                idx = (slice(None), pl.ds(mult((p * SLAB_PER + t) * WO_SLAB, 8), WO_SLAB), slice(None))
                pltpu.make_async_copy(wo_hbm.at[idx], wo_v.at[idx], sem.at[S_WO]).start()
        else:
            idx = (pl.ds(2 * p, 2),)
            pltpu.make_async_copy(wo_hbm.at[idx], wo_v.at[idx], sem.at[S_WO]).start()

    wo_all = pltpu.make_async_copy(wo_hbm, wo_v, sem.at[S_WO])
    w1_cp = pltpu.make_async_copy(w1_hbm, w1_v, sem.at[S_W1])

    def w2_cp(j):
        sl = pl.ds(W2_BOUNDS[j], W2_BOUNDS[j + 1] - W2_BOUNDS[j])
        return pltpu.make_async_copy(w2_hbm.at[sl, :], w2_v.at[sl, :], sem.at[S_W2 + j])

    def side_a(j, inbound):
        slot = lax.rem(j, NS)
        rt = lax.div(j, 2)
        idx = (lax.div(rt, MR // 8), pl.ds(mult(lax.rem(rt, MR // 8) * 8, 8), 8),
               pl.ds(mult(2 * D + lax.rem(j, 2) * A_COLS, 128), A_COLS))
        if inbound:
            return pltpu.make_async_copy(wmod_hbm.at[idx], sa_s.at[slot], sem.at[S_IN + slot])
        return pltpu.make_async_copy(sa_s.at[slot], wmod_v.at[idx], sem.at[S_SV + slot])

    def side_b(j, inbound):
        slot = lax.rem(j, NS)
        r = pl.ds(mult((j - NA) * B_ROWS, 8), B_ROWS)
        if inbound:
            return pltpu.make_async_copy(w2_hbm.at[r, :], sb_s.at[slot], sem.at[S_IN + slot])
        return pltpu.make_async_copy(sb_s.at[slot], w2_v.at[r, :], sem.at[S_SV + slot])

    def side_do(j, inbound, op):
        @pl.when(jnp.logical_and(j >= 0, j < NA))
        def _():
            op(side_a(j, inbound))

        if NB:
            @pl.when(jnp.logical_and(j >= NA, j < NSIDE))
            def _():
                op(side_b(j, inbound))

    start = lambda d: d.start()
    wait = lambda d: d.wait()

    def side_event(j, carry):
        side_do(j, True, wait)
        side_do(j, False, start)
        side_do(j - LAG, False, wait)
        side_do(j - LAG + NS, True, start)
        return carry

    def side_events(j0, j1):
        if isinstance(j0, int) and isinstance(j1, int):
            j1 = min(j1, NSIDE + LAG)
            if j0 >= j1:
                return
            j0, j1 = jnp.int32(j0), jnp.int32(j1)
        else:
            j1 = jnp.minimum(j1, NSIDE + LAG)
        lax.fori_loop(j0, j1, side_event, 0)

    if MSLAB:
        wma_cp(0, 8).start()
    else:
        wma_cp(0, MR).start()
    c_cp.start()
    x_cp.start()
    for j in range(NS - LAG):
        side_a(jnp.int32(j), True).start()
    if MSLAB:
        for i in range(1, MR // 8):
            wma_cp(i, 8).start()
    def wq_start(j):
        if QSLAB:
            for i in range(QR // 8):
                wq_cp(j, i, 8).start()
        else:
            wq_cp(j, 0, QR).start()

    def pair_start(p):
        kv_start(k_hbm, p, 2 * p)
        kv_start(v_hbm, p, 2 * p + 1)
        wo_start(p)

    def tail_start():
        b1_cp.start(priority=1)
        w1_cp.start(priority=1)
        for j in range(NW2):
            w2_cp(j).start(priority=1)

    todo = [functools.partial(wq_start, j) for j in range(WQ_CHUNKS)]
    todo += [functools.partial(pair_start, p) for p in range(AHEAD)] + [tail_start]
    stages = (2, 1, 1, 2, 2, 1)
    assert sum(stages) == len(todo)

    def issue_stage(k):
        for _ in range(stages[k]):
            todo.pop(0)()

    issue_stage(0)

    c_cp.wait()
    x_cp.wait()
    c32 = c_v[...].astype(f32)
    sc = c32 * jax.nn.sigmoid(c32)
    sc8 = jnp.broadcast_to(sc, (8, D)).astype(bf16)
    x32 = x_v[...].astype(f32)
    xn = _layernorm(x32)
    acc_s[...] = jnp.zeros((8, D), f32)
    ev = 0
    side_events(ev, ev + PRE[0])
    ev += PRE[0]
    wma_cp(0, MR).wait()
    issue_stage(1)
    mod_a = jnp.dot(sc8, wmod_v[:, :, 0:2 * D].reshape(D, 2 * D), preferred_element_type=f32)
    h = xn * (1.0 + mod_a[:, D:2 * D]) + mod_a[:, 0:D]
    h8 = h.astype(bf16)

    row = lax.broadcasted_iota(jnp.int32, (8, PAIR), 0)
    lane = lax.broadcasted_iota(jnp.int32, (8, PAIR), 1)
    diag = (row == jnp.where(lane >= DH, 1, 0))
    ppc = NPAIR // WQ_CHUNKS
    for j in range(WQ_CHUNKS):
        n_ev = sum(PRE[1:5]) * (j + 1) // WQ_CHUNKS - sum(PRE[1:5]) * j // WQ_CHUNKS
        side_events(ev, ev + n_ev)
        ev += n_ev
        wq_cp(j, 0, QR).wait()
        issue_stage(2 + j)
        wqj = wq_v[:, :, j * wq_cols:(j + 1) * wq_cols].reshape(D, wq_cols)
        qj = jnp.dot(h8, wqj, preferred_element_type=f32)
        for t in range(ppc):
            q_s[j * ppc + t] = jnp.where(diag, qj[:, t * PAIR:(t + 1) * PAIR], 0.0)
    side_events(ev, ev + PRE[5])
    ev += PRE[5]
    ev0 = ev

    def ev_at(p, half):
        mn = min(p, 8) if isinstance(p, int) else jnp.minimum(p, 8)
        return ev0 + (p * R_PAIR + mn * R_SLAB + half * R_V + PHASE) // 256

    scale = DH ** -0.5

    def pair_step(p, carry):
        slot = lax.rem(p, AHEAD)
        ks = 2 * slot
        vs = ks + 1
        kv_wait(k_hbm, p, ks)
        q2 = q_s[p].astype(bf16)
        s = jnp.concatenate([jnp.dot(q2, kv_buf[ks, t], preferred_element_type=f32)
                             for t in range(KVSPLIT)], axis=1) * scale

        @pl.when(p + AHEAD < NPAIR)
        def _():
            kv_start(k_hbm, p + AHEAD, ks)

        m = jnp.max(s, axis=-1, keepdims=True)
        e = jnp.exp(s - m)
        l = jnp.sum(e, axis=-1, keepdims=True)
        e16 = e.astype(bf16)

        @pl.when(p == MODB_AT)
        def _():
            modb_s[...] = jnp.dot(sc8, wmod_v[:, :, 2 * D:6 * D].reshape(D, 4 * D), preferred_element_type=f32)

        @pl.when(p == 8)
        def _():
            wo_all.wait()

        @pl.when(p >= 8)
        def _():
            acc_s[...] += jnp.dot(o_s[p - 8].astype(bf16), wo_v[p - 8], preferred_element_type=f32)

        side_events(ev_at(p, 0), ev_at(p, 1))
        kv_wait(v_hbm, p, vs)
        o2 = sum(lax.dot_general(e16[:, t * wc:(t + 1) * wc], kv_buf[vs, t], (((1,), (1,)), ((), ())),
                                 preferred_element_type=f32) for t in range(KVSPLIT))
        o2 = jnp.where(diag, o2 / l, 0.0)

        @pl.when(p + AHEAD < NPAIR)
        def _():
            kv_start(v_hbm, p + AHEAD, vs)

        @pl.when(p + AHEAD < 8)
        def _():
            wo_start(p + AHEAD)

        @pl.when(p < 8)
        def _():
            o_s[p] = o2

        @pl.when(p >= 8)
        def _():
            acc_s[...] += jnp.dot(o2.astype(bf16), wo_v[p], preferred_element_type=f32)

        @pl.when(p + 1 < NPAIR)
        def _():
            side_events(ev_at(p, 1), ev_at(p + 1, 0))

        return carry

    assert ev_at(MODB_AT, 0) >= NA + LAG, "w_mod must be resident before it is used"
    assert ev_at(0, 0) == ev0
    lax.fori_loop(0, NPAIR, pair_step, 0)
    attn = jnp.sum(acc_s[...], axis=0, keepdims=True)
    ev = ev_at(NPAIR - 1, 1)

    ga, sb, cb, gb = (modb_s[:, i * D:(i + 1) * D] for i in range(4))
    x1 = x32 + ga * attn

    h2 = (_layernorm(x1) * (1.0 + cb) + sb).astype(bf16)
    b1_cp.wait()
    b1 = b1_v[...].astype(f32)
    b1row = jnp.concatenate([b1[j:j + 1, :] for j in range(F // 128)], axis=1)
    side_events(ev, ev + POST[0])
    ev += POST[0]
    w1_cp.wait()
    u = jnp.dot(h2, w1_v[...], preferred_element_type=f32) + b1row
    sp = jnp.log1p(jnp.exp(-jnp.abs(u))) + jnp.maximum(u, 0.0)
    act = (u * jnp.tanh(sp)).astype(bf16)
    y = jnp.zeros((8, D), f32)
    for j in range(NW2):
        w2_cp(j).wait()
        o0 = max(W2_BOUNDS[j], SIDE_K)
        o1 = W2_BOUNDS[j + 1]
        if o1 > o0:
            y = y + jnp.dot(act[:, o0:o1], w2_v[o0:o1, :], preferred_element_type=f32)
        if j == SIDE_AFTER:
            side_events(ev, NSIDE + LAG)
            if SIDE_K:
                y = y + jnp.dot(act[:, 0:SIDE_K], w2_v[0:SIDE_K, :], preferred_element_type=f32)
    res = x1 + gb * y
    out_v[...] = res[0:1, :].astype(bf16)
    out_cp = pltpu.make_async_copy(out_v, out_hbm, sem.at[S_OUT])
    out_cp.start()
    out_cp.wait()


@jax.jit
def pallas_adaLN_cond__sliding_block_cached__dense_activation_mish__decode_kernel(
    A_x: jax.Array,
    A_k_cache: jax.Array,
    A_v_cache: jax.Array,
    A_wq: jax.Array,
    A_wo: jax.Array,
    B_x: jax.Array,
    B_w1: jax.Array,
    B_b1: jax.Array,
    B_w2: jax.Array,
    c: jax.Array,
    w_mod: jax.Array,
):
    del B_x
    SK = A_k_cache.shape[2]
    W = min(4096, max(256, SK // 4))
    kt = jnp.swapaxes(A_k_cache, 2, 3).reshape(H * DH, SK)
    vt = jnp.swapaxes(A_v_cache, 2, 3).reshape(H * DH, SK)
    x = A_x.reshape(1, D)
    b1 = B_b1.reshape(F // 128, 128)
    wm3 = w_mod.reshape(MG, MR, 6 * D)
    wq3 = A_wq.reshape(QG, QR, H * DH)
    wo3 = A_wo.reshape(NPAIR, PAIR, D)

    any_spec = pl.BlockSpec(memory_space=pl.ANY)
    out = pl.pallas_call(
        functools.partial(_kernel, W=W, SK=SK),
        out_shape=jax.ShapeDtypeStruct((1, D), bf16),
        in_specs=[any_spec] * 10,
        out_specs=any_spec,
        scratch_shapes=[
            pltpu.VMEM((1, D), bf16),
            pltpu.VMEM((1, D), bf16),
            pltpu.VMEM((F // 128, 128), bf16),
            pltpu.VMEM((MG, MR, 6 * D), bf16),
            pltpu.VMEM((QG, QR, H * DH), bf16),
            pltpu.VMEM((NBUF, KVSPLIT, PAIR, W // KVSPLIT), bf16),
            pltpu.VMEM((NPAIR, PAIR, D), bf16),
            pltpu.VMEM((D, F), bf16),
            pltpu.VMEM((F, D), bf16),
            pltpu.VMEM((NPAIR, 8, PAIR), f32),
            pltpu.VMEM((8, 8, PAIR), f32),
            pltpu.VMEM((8, D), f32),
            pltpu.VMEM((8, 4 * D), f32),
            pltpu.VMEM((1, D), bf16),
            pltpu.SMEM((NS, 8, A_COLS), bf16),
            pltpu.SMEM((NS, B_ROWS, D), bf16),
            pltpu.SemaphoreType.DMA((NSEM,)),
        ],
        compiler_params=pltpu.CompilerParams(
            vmem_limit_bytes=100 * 1024 * 1024,
            disable_bounds_checks=True,
            disable_semaphore_checks=True,
        ),
    )(x, c, b1, wm3, wq3, kt, vt, wo3, B_w1, B_w2)
    return out.reshape(1, 1, D)
```

```python
import functools

import jax
import jax.numpy as jnp
from jax import lax
import jax.experimental.pallas as pl
import jax.experimental.pallas.tpu as pltpu

D = 640
H = 32
DH = 192
F = 1536
PAIR = 2 * DH
NPAIR = H // 2
AHEAD = 2
NBUF = 2 * AHEAD
EPS = 1e-5

MG, MR = 10, 64
QG, QR = 8, 80
QC = 2048
NQC = H * DH // QC
KVS = (1024, 1024, 2048)

QK_CH = 512
PV_CH = 256
N1 = 41
D1 = 50
D2 = 50
DP = 43
DP2 = 66
PPP = 96
PRO = (27, 39, 39, 39, 26, 35)
SL = 4
BULK0 = 10
W2_END = (768, 1152, 1408, 1536)

f32 = jnp.float32
bf16 = jnp.bfloat16

S_C, S_X, S_B1, S_WMA, S_WMB, S_W1, S_W1P, S_W2P, S_OUT = range(9)
S_WO = 9
S_WQ = S_WO + 2
S_W2 = S_WQ + NQC
S_KV = S_W2 + len(W2_END)
NSEM = S_KV + NBUF


def _layernorm(x):
    m = jnp.mean(x, axis=-1, keepdims=True)
    xc = x - m
    v = jnp.mean(xc * xc, axis=-1, keepdims=True)
    return xc / jnp.sqrt(v + EPS)


def _kernel(x_hbm, c_hbm, b1_hbm, wmod_hbm, wq_hbm, k_hbm, v_hbm, wo_hbm, w1_hbm, w2_hbm,
            out_hbm,
            x_v, c_v, b1_v, wmod_v, wq_v, kv_buf, wo_v, w1_v, w2_v, q_s, s_s, e_s, mod_s, out_v, sem,
            *, W, SK):
    col0 = SK - W
    nqk = W // QK_CH
    npv = W // PV_CH
    n2 = PPP - nqk - npv - N1
    w2_pieces = (nqk + N1 + npv) // 2 * 2
    w2_rows = 4 * w2_pieces

    def mult(v, m):
        return v if isinstance(v, int) else pl.multiple_of(v, m)

    def copy(src, dst, s):
        return pltpu.make_async_copy(src, dst, sem.at[s])

    def ticks(n, tick, delay):
        def body(i, carry):
            tick(i)
            pl.delay(delay)
            return carry
        lax.fori_loop(0, n, body, 0)

    def wm_cp(i, c0, s, n=8, nc=2 * D):
        idx = (slice(None), pl.ds(mult(8 * i, 8), n), pl.ds(mult(c0, 128), nc))
        return copy(wmod_hbm.at[idx], wmod_v.at[idx], s)

    def wq_cp(j, i, n=8):
        idx = (slice(None), pl.ds(mult(8 * i, 8), n), pl.ds(mult(j * QC, 128), QC))
        return copy(wq_hbm.at[idx], wq_v.at[idx], S_WQ + j)

    def kv_cps(src, p, slot):
        rows = pl.ds(mult(p * PAIR, PAIR), PAIR)
        offs = [sum(KVS[:t]) for t in range(len(KVS))]
        return [copy(src.at[rows, pl.ds(col0 + o, n)], kv_buf.at[slot, :, pl.ds(o, n)], S_KV + slot)
                for o, n in zip(offs, KVS)]

    def kv_start(src, p, slot):
        for d in kv_cps(src, p, slot):
            d.start(priority=1)

    def kv_wait(src, p, slot):
        copy(kv_buf.at[slot], kv_buf.at[slot], S_KV + slot).wait()

    n_wma, n_wq, n_wmb = MR // 8, NQC * (QR // 8), 2 * (MR // 8)
    n_slab = n_wma + n_wq + n_wmb

    def slab_start(i):
        if isinstance(i, int):
            if i < n_wma:
                wm_cp(i, 0, S_WMA).start(priority=1)
            elif i < n_wma + n_wq:
                wq_cp((i - n_wma) // (QR // 8), (i - n_wma) % (QR // 8)).start(priority=1)
            else:
                k = i - n_wma - n_wq
                wm_cp(k // 2, 2 * D + (k % 2) * 2 * D, S_WMB).start(priority=1)
            return

        @pl.when(i < n_wma + n_wq)
        def _():
            k = i - n_wma
            wq_cp(lax.div(k, QR // 8), lax.rem(k, QR // 8)).start(priority=1)

        @pl.when(jnp.logical_and(i >= n_wma + n_wq, i < n_slab))
        def _():
            k = i - n_wma - n_wq
            wm_cp(lax.div(k, 2), 2 * D + lax.rem(k, 2) * 2 * D, S_WMB).start(priority=1)

    def row_piece(src, dst, j, s):
        r = pl.ds(mult(lax.div(j, 2) * 8, 8), 8)

        @pl.when(lax.rem(j, 2) == 0)
        def _():
            copy(src.at[r, pl.ds(0, PAIR)], dst.at[r, pl.ds(0, PAIR)], s).start()

        @pl.when(lax.rem(j, 2) == 1)
        def _():
            copy(src.at[r, pl.ds(PAIR, D - PAIR)], dst.at[r, pl.ds(PAIR, D - PAIR)], s).start()

    def w1_piece(j):
        idx = (pl.ds(mult(lax.div(j, 4) * 8, 8), 8), pl.ds(mult(lax.rem(j, 4) * PAIR, 128), PAIR))
        copy(w1_hbm.at[idx], w1_v.at[idx], S_W1P).start()

    n_pro = sum(PRO) + 5 + NPAIR + 10
    w1_pieces = (n_pro - PPP) // 4 * 4
    w1_rows = 2 * w1_pieces

    def pro_piece(j):
        @pl.when(j < w1_pieces)
        def _():
            w1_piece(j)

        @pl.when(jnp.logical_and(j >= w1_pieces, j < w1_pieces + PPP))
        def _():
            row_piece(wo_hbm.at[0], wo_v.at[0], j - w1_pieces, S_WO)

    def loop_piece(p, j):
        @pl.when(p + 1 < NPAIR)
        def _():
            nxt = lax.rem(p + 1, 2)
            row_piece(wo_hbm.at[p + 1], wo_v.at[nxt], j, S_WO + nxt)

        @pl.when(jnp.logical_and(p + 1 == NPAIR, j < w2_pieces))
        def _():
            row_piece(w2_hbm, w2_v, j, S_W2P)

    w1_cp = copy(w1_hbm.at[pl.ds(w1_rows, D - w1_rows), :], w1_v.at[pl.ds(w1_rows, D - w1_rows), :], S_W1)
    w2_bounds = [w2_rows] + list(W2_END)

    def w2_cp(j):
        sl = pl.ds(w2_bounds[j], w2_bounds[j + 1] - w2_bounds[j])
        return copy(w2_hbm.at[sl, :], w2_v.at[sl, :], S_W2 + j)

    x_cp = copy(x_hbm, x_v, S_X)
    c_cp = copy(c_hbm, c_v, S_C)
    b1_cp = copy(b1_hbm, b1_v, S_B1)
    slab_start(0)
    c_cp.start()
    x_cp.start()
    for i in range(1, BULK0):
        slab_start(i)
    b1_cp.start()

    state = {"piece": 0, "slab": BULK0}

    def pro_idle(n):
        j0, i0 = state["piece"], state["slab"]

        def tick(i):
            pro_piece(j0 + i)

            if i0 < n_slab:
                @pl.when(lax.rem(i, SL) == 0)
                def _():
                    slab_start(i0 + lax.div(i, SL))

        ticks(n, tick, DP if i0 < n_slab else DP2)
        state["piece"] += n
        state["slab"] += -(-n // SL)

    def pro_compute(n, step):
        j0, i0 = state["piece"], state["slab"]

        def body(i, carry):
            pro_piece(j0 + i)

            if i0 < n_slab:
                @pl.when(lax.rem(i, 2) == 0)
                def _():
                    slab_start(i0 + lax.div(i, 2))

            step(i)
            return carry

        lax.fori_loop(0, n, body, 0)
        state["piece"] += n
        state["slab"] += -(-n // 2)

    pro_idle(PRO[0])
    c_cp.wait()
    x_cp.wait()
    c32 = c_v[...].astype(f32)
    sc = c32 * jax.nn.sigmoid(c32)
    sc8 = jnp.broadcast_to(sc, (8, D)).astype(bf16)
    x32 = x_v[...].astype(f32)
    xn = _layernorm(x32)

    def mod_step(first):
        def step(i):
            cs = pl.ds(pl.multiple_of((first + i) * 256, 256), 256)
            mod_s[:, cs] = jnp.dot(sc8, wmod_v[:, :, cs].reshape(D, 256), preferred_element_type=f32)
        return step

    wm_cp(0, 0, S_WMA, n=MR).wait()
    pro_compute(5, mod_step(0))
    h = xn * (1.0 + mod_s[:, D:2 * D]) + mod_s[:, 0:D]
    h8 = h.astype(bf16)

    row = lax.broadcasted_iota(jnp.int32, (8, PAIR), 0)
    lane = lax.broadcasted_iota(jnp.int32, (8, PAIR), 1)
    diag = (row == jnp.where(lane >= DH, 1, 0))

    for j in range(3):
        pro_idle(PRO[1 + j])
    assert state["slab"] >= n_wma + n_wq, state
    for j in range(NQC):
        wq_cp(j, 0, n=QR).wait()

    def q_step(p):
        cs = pl.ds(pl.multiple_of(p * PAIR, 128), PAIR)
        qp = jnp.dot(h8, wq_v[:, :, cs].reshape(D, PAIR), preferred_element_type=f32)
        q_s[p] = jnp.where(diag, qp, 0.0)

    pro_compute(NPAIR, q_step)
    assert state["slab"] >= n_slab, state
    kv_start(k_hbm, 0, 0)
    kv_start(v_hbm, 0, 1)
    pro_idle(PRO[4])
    wm_cp(0, 2 * D, S_WMB, n=MR, nc=4 * D).wait()
    kv_start(k_hbm, 1, 2)
    kv_start(v_hbm, 1, 3)
    pro_compute(10, mod_step(5))
    pro_idle(PRO[5])
    assert state["piece"] == n_pro

    scale = DH ** -0.5

    def pair_step(p, acc):
        slot = lax.rem(p, AHEAD)
        ks = 2 * slot
        vs = ks + 1
        kv_wait(k_hbm, p, ks)
        q2 = q_s[p].astype(bf16)

        def qk_body(i, carry):
            loop_piece(p, i)
            kc = kv_buf[ks, :, pl.ds(pl.multiple_of(i * QK_CH, 128), QK_CH)]
            s_s[:, pl.ds(pl.multiple_of(i * QK_CH, 128), QK_CH)] = jnp.dot(q2, kc, preferred_element_type=f32)
            return carry

        lax.fori_loop(0, nqk, qk_body, 0)

        @pl.when(p + AHEAD < NPAIR)
        def _():
            kv_start(k_hbm, p + AHEAD, ks)

        s = s_s[...] * scale
        m = jnp.max(s, axis=-1, keepdims=True)
        e = jnp.exp(s - m)
        l = jnp.sum(e, axis=-1, keepdims=True)
        e_s[...] = e

        ticks(N1, lambda i: loop_piece(p, nqk + i), D1)
        kv_wait(v_hbm, p, vs)

        def pv_body(i, o2):
            loop_piece(p, nqk + N1 + i)
            vc = kv_buf[vs, :, pl.ds(pl.multiple_of(i * PV_CH, 128), PV_CH)]
            ec = e_s[:, pl.ds(pl.multiple_of(i * PV_CH, 128), PV_CH)].astype(bf16)
            return o2 + lax.dot_general(ec, vc, (((1,), (1,)), ((), ())), preferred_element_type=f32)

        o2 = lax.fori_loop(0, npv, pv_body, jnp.zeros((8, PAIR), f32))

        @pl.when(p + AHEAD < NPAIR)
        def _():
            kv_start(v_hbm, p + AHEAD, vs)

        @pl.when(p + AHEAD == NPAIR - 1)
        def _():
            w1_cp.start(priority=1)
            for j in range(len(W2_END)):
                w2_cp(j).start(priority=1)

        o2 = jnp.where(diag, o2 / l, 0.0).astype(bf16)
        cur = lax.rem(p, 2)
        copy(wo_v.at[cur], wo_v.at[cur], S_WO + cur).wait()
        acc = acc + jnp.dot(o2, wo_v[cur], preferred_element_type=f32)

        ticks(jnp.where(p + 1 < NPAIR, n2, 0), lambda i: loop_piece(p, nqk + N1 + npv + i), D2)
        return acc

    acc = lax.fori_loop(0, NPAIR, pair_step, jnp.zeros((8, D), f32))
    attn = jnp.sum(acc, axis=0, keepdims=True)

    ga, sb, cb, gb = (mod_s[:, i * D:(i + 1) * D] for i in range(2, 6))
    x1 = x32 + ga * attn

    h2 = (_layernorm(x1) * (1.0 + cb) + sb).astype(bf16)
    b1_cp.wait()
    b1 = b1_v[...].astype(f32)
    b1row = jnp.concatenate([b1[j:j + 1, :] for j in range(F // 128)], axis=1)
    copy(w1_v.at[pl.ds(0, w1_rows), :], w1_v.at[pl.ds(0, w1_rows), :], S_W1P).wait()
    w1_cp.wait()
    u = jnp.dot(h2, w1_v[...], preferred_element_type=f32) + b1row
    sp = jnp.log1p(jnp.exp(-jnp.abs(u))) + jnp.maximum(u, 0.0)
    act = (u * jnp.tanh(sp)).astype(bf16)
    copy(w2_v.at[pl.ds(0, w2_rows), :], w2_v.at[pl.ds(0, w2_rows), :], S_W2P).wait()
    y = jnp.zeros((8, D), f32)
    for j in range(len(W2_END)):
        w2_cp(j).wait()
        o0 = 0 if j == 0 else W2_END[j - 1]
        o1 = W2_END[j]
        y = y + jnp.dot(act[:, o0:o1], w2_v[o0:o1, :], preferred_element_type=f32)
    res = x1 + gb * y
    out_v[...] = res[0:1, :].astype(bf16)
    out_cp = copy(out_v, out_hbm, S_OUT)
    out_cp.start()
    out_cp.wait()


@jax.jit
def pallas_adaLN_cond__sliding_block_cached__dense_activation_mish__decode_kernel(
    A_x: jax.Array,
    A_k_cache: jax.Array,
    A_v_cache: jax.Array,
    A_wq: jax.Array,
    A_wo: jax.Array,
    B_x: jax.Array,
    B_w1: jax.Array,
    B_b1: jax.Array,
    B_w2: jax.Array,
    c: jax.Array,
    w_mod: jax.Array,
):
    del B_x
    SK = A_k_cache.shape[2]
    W = min(4096, max(256, SK // 4))
    kt = jnp.swapaxes(A_k_cache, 2, 3).reshape(H * DH, SK)
    vt = jnp.swapaxes(A_v_cache, 2, 3).reshape(H * DH, SK)
    x = A_x.reshape(1, D)
    b1 = B_b1.reshape(F // 128, 128)
    wm3 = w_mod.reshape(MG, MR, 6 * D)
    wq3 = A_wq.reshape(QG, QR, H * DH)
    wo3 = A_wo.reshape(NPAIR, PAIR, D)

    any_spec = pl.BlockSpec(memory_space=pl.ANY)
    out = pl.pallas_call(
        functools.partial(_kernel, W=W, SK=SK),
        out_shape=jax.ShapeDtypeStruct((1, D), bf16),
        in_specs=[any_spec] * 10,
        out_specs=any_spec,
        scratch_shapes=[
            pltpu.VMEM((1, D), bf16),
            pltpu.VMEM((1, D), bf16),
            pltpu.VMEM((F // 128, 128), bf16),
            pltpu.VMEM((MG, MR, 6 * D), bf16),
            pltpu.VMEM((QG, QR, H * DH), bf16),
            pltpu.VMEM((NBUF, PAIR, W), bf16),
            pltpu.VMEM((2, PAIR, D), bf16),
            pltpu.VMEM((D, F), bf16),
            pltpu.VMEM((F, D), bf16),
            pltpu.VMEM((NPAIR, 8, PAIR), f32),
            pltpu.VMEM((8, W), f32),
            pltpu.VMEM((8, W), f32),
            pltpu.VMEM((8, 6 * D), f32),
            pltpu.VMEM((1, D), bf16),
            pltpu.SemaphoreType.DMA((NSEM,)),
        ],
        compiler_params=pltpu.CompilerParams(
            vmem_limit_bytes=100 * 1024 * 1024,
            disable_bounds_checks=True,
            disable_semaphore_checks=True,
        ),
    )(x, c, b1, wm3, wq3, kt, vt, wo3, B_w1, B_w2)
    return out.reshape(1, 1, D)
```

```python
import functools

import jax
import jax.numpy as jnp
from jax import lax
import jax.experimental.pallas as pl
import jax.experimental.pallas.tpu as pltpu

D = 640
H = 32
DH = 192
F = 1536
PAIR = 2 * DH
NPAIR = H // 2
AHEAD = 2
NBUF = 2 * AHEAD
EPS = 1e-5

MG, MR = 10, 64
QG, QR = 8, 80
QC = 2048
NQC = H * DH // QC
KVS = (1024, 1024, 2048)

T1 = 8
TPV = 16
TWO = 2
T2 = TPV + TWO
N1 = 38
D1 = 82
D2 = 82
DP = 43
DP2 = 66
PPP = 96
PRO = (27, 39, 39, 39, 26, 35)
SL = 4
BULK0 = 10
NW2 = 5

f32 = jnp.float32
bf16 = jnp.bfloat16

S_C, S_X, S_B1, S_WMA, S_WMB, S_W1, S_W1P, S_W2P, S_OUT = range(9)
S_WO = 9
S_WQ = S_WO + 2
S_W2 = S_WQ + NQC
S_KV = S_W2 + NW2
NSEM = S_KV + NBUF


def _layernorm(x):
    m = jnp.mean(x, axis=-1, keepdims=True)
    xc = x - m
    v = jnp.mean(xc * xc, axis=-1, keepdims=True)
    return xc / jnp.sqrt(v + EPS)


def _kernel(x_hbm, c_hbm, b1_hbm, wmod_hbm, wq_hbm, k_hbm, v_hbm, wo_hbm, w1_hbm, w2_hbm,
            out_hbm,
            x_v, c_v, b1_v, wmod_v, wq_v, big, w1_v, q_s, mod_s, out_v, sem,
            *, W, SK):
    col0 = SK - W
    n2 = PPP - T1 - T2 - N1
    assert T1 % 2 == 0 and N1 % 2 == 0 and T2 % 2 == 0
    w2_pieces = T1 + N1 + T2
    w2_rows = 4 * w2_pieces

    def kv_ref(slot):
        return big.at[slot, :, pl.ds(0, W)]

    def wo_ref(slot):
        return big.at[slot, :, pl.ds(W, D)]

    def w2_ref(g):
        return big.at[g, :, pl.ds(W + D, D)]

    def mult(v, m):
        return v if isinstance(v, int) else pl.multiple_of(v, m)

    def copy(src, dst, s):
        return pltpu.make_async_copy(src, dst, sem.at[s])

    def ticks(n, tick, delay):
        def body(i, carry):
            tick(i)
            pl.delay(delay)
            return carry
        lax.fori_loop(0, n, body, 0)

    def wm_cp(i, c0, s, n=8, nc=2 * D):
        idx = (slice(None), pl.ds(mult(8 * i, 8), n), pl.ds(mult(c0, 128), nc))
        return copy(wmod_hbm.at[idx], wmod_v.at[idx], s)

    def wq_cp(j, i, n=8):
        idx = (slice(None), pl.ds(mult(8 * i, 8), n), pl.ds(mult(j * QC, 128), QC))
        return copy(wq_hbm.at[idx], wq_v.at[idx], S_WQ + j)

    def kv_cps(src, p, slot):
        rows = pl.ds(mult(p * PAIR, PAIR), PAIR)
        offs = [sum(KVS[:t]) for t in range(len(KVS))]
        return [copy(src.at[rows, pl.ds(col0 + o, n)], big.at[slot, :, pl.ds(o, n)], S_KV + slot)
                for o, n in zip(offs, KVS)]

    def kv_start(src, p, slot):
        for d in kv_cps(src, p, slot):
            d.start(priority=1)

    def kv_wait(src, p, slot):
        copy(kv_ref(slot), kv_ref(slot), S_KV + slot).wait()

    n_wma, n_wq, n_wmb = MR // 8, NQC * (QR // 8), 2 * (MR // 8)
    n_slab = n_wma + n_wq + n_wmb

    def slab_start(i):
        if isinstance(i, int):
            if i < n_wma:
                wm_cp(i, 0, S_WMA).start(priority=1)
            elif i < n_wma + n_wq:
                wq_cp((i - n_wma) // (QR // 8), (i - n_wma) % (QR // 8)).start(priority=1)
            else:
                k = i - n_wma - n_wq
                wm_cp(k // 2, 2 * D + (k % 2) * 2 * D, S_WMB).start(priority=1)
            return

        @pl.when(i < n_wma + n_wq)
        def _():
            k = i - n_wma
            wq_cp(lax.div(k, QR // 8), lax.rem(k, QR // 8)).start(priority=1)

        @pl.when(jnp.logical_and(i >= n_wma + n_wq, i < n_slab))
        def _():
            k = i - n_wma - n_wq
            wm_cp(lax.div(k, 2), 2 * D + lax.rem(k, 2) * 2 * D, S_WMB).start(priority=1)

    def row_piece(src, dst, j, s):
        if isinstance(j, int):
            r = pl.ds((j // 2) * 8, 8)
            cs = pl.ds(0, PAIR) if j % 2 == 0 else pl.ds(PAIR, D - PAIR)
            copy(src.at[r, cs], dst.at[r, cs], s).start()
            return
        r = pl.ds(mult(lax.div(j, 2) * 8, 8), 8)

        @pl.when(lax.rem(j, 2) == 0)
        def _():
            copy(src.at[r, pl.ds(0, PAIR)], dst.at[r, pl.ds(0, PAIR)], s).start()

        @pl.when(lax.rem(j, 2) == 1)
        def _():
            copy(src.at[r, pl.ds(PAIR, D - PAIR)], dst.at[r, pl.ds(PAIR, D - PAIR)], s).start()

    def w1_piece(j):
        idx = (pl.ds(mult(lax.div(j, 4) * 8, 8), 8), pl.ds(mult(lax.rem(j, 4) * PAIR, 128), PAIR))
        copy(w1_hbm.at[idx], w1_v.at[idx], S_W1P).start()

    n_pro = sum(PRO) + 5 + NPAIR + 10
    w1_pieces = (n_pro - PPP) // 4 * 4
    w1_rows = 2 * w1_pieces

    def pro_piece(j):
        @pl.when(j < w1_pieces)
        def _():
            w1_piece(j)

        @pl.when(jnp.logical_and(j >= w1_pieces, j < w1_pieces + PPP))
        def _():
            row_piece(wo_hbm.at[0], wo_ref(0), j - w1_pieces, S_WO)

    def loop_piece(p, j):
        @pl.when(p + 1 < NPAIR)
        def _():
            nxt = lax.rem(p + 1, 2)
            row_piece(wo_hbm.at[p + 1], wo_ref(nxt), j, S_WO + nxt)

        @pl.when(p + 1 == NPAIR)
        def _():
            row_piece(w2_hbm.at[0], w2_ref(0), j, S_W2P)

    w1_cp = copy(w1_hbm.at[pl.ds(w1_rows, D - w1_rows), :], w1_v.at[pl.ds(w1_rows, D - w1_rows), :], S_W1)
    w2_parts = [(0, w2_rows, PAIR), (1, 0, PAIR), (2, 0, PAIR), (3, 0, 256), (3, 256, PAIR)]

    def w2_cp(j):
        g, r0, r1 = w2_parts[j]
        sl = pl.ds(r0, r1 - r0)
        return copy(w2_hbm.at[g, sl, :], w2_ref(g).at[sl, :], S_W2 + j)

    x_cp = copy(x_hbm, x_v, S_X)
    c_cp = copy(c_hbm, c_v, S_C)
    b1_cp = copy(b1_hbm, b1_v, S_B1)
    slab_start(0)
    c_cp.start()
    x_cp.start()
    for i in range(1, BULK0):
        slab_start(i)
    b1_cp.start()

    state = {"piece": 0, "slab": BULK0}

    def pro_idle(n):
        j0, i0 = state["piece"], state["slab"]

        def tick(i):
            pro_piece(j0 + i)

            if i0 < n_slab:
                @pl.when(lax.rem(i, SL) == 0)
                def _():
                    slab_start(i0 + lax.div(i, SL))

        ticks(n, tick, DP if i0 < n_slab else DP2)
        state["piece"] += n
        state["slab"] += -(-n // SL)

    def pro_compute(n, step):
        j0, i0 = state["piece"], state["slab"]

        def body(i, carry):
            pro_piece(j0 + i)

            if i0 < n_slab:
                @pl.when(lax.rem(i, 2) == 0)
                def _():
                    slab_start(i0 + lax.div(i, 2))

            step(i)
            return carry

        lax.fori_loop(0, n, body, 0)
        state["piece"] += n
        state["slab"] += -(-n // 2)

    pro_idle(PRO[0])
    c_cp.wait()
    x_cp.wait()
    c32 = c_v[...].astype(f32)
    sc = c32 * jax.nn.sigmoid(c32)
    sc8 = jnp.broadcast_to(sc, (8, D)).astype(bf16)
    x32 = x_v[...].astype(f32)
    xn = _layernorm(x32)

    def mod_step(first):
        def step(i):
            cs = pl.ds(pl.multiple_of((first + i) * 256, 256), 256)
            mod_s[:, cs] = jnp.dot(sc8, wmod_v[:, :, cs].reshape(D, 256), preferred_element_type=f32)
        return step

    wm_cp(0, 0, S_WMA, n=MR).wait()
    pro_compute(5, mod_step(0))
    h = xn * (1.0 + mod_s[:, D:2 * D]) + mod_s[:, 0:D]
    h8 = h.astype(bf16)

    row = lax.broadcasted_iota(jnp.int32, (8, PAIR), 0)
    lane = lax.broadcasted_iota(jnp.int32, (8, PAIR), 1)
    diag = (row == jnp.where(lane >= DH, 1, 0))

    for j in range(3):
        pro_idle(PRO[1 + j])
    assert state["slab"] >= n_wma + n_wq, state
    for j in range(NQC):
        wq_cp(j, 0, n=QR).wait()

    def q_step(p):
        cs = pl.ds(pl.multiple_of(p * PAIR, 128), PAIR)
        qp = jnp.dot(h8, wq_v[:, :, cs].reshape(D, PAIR), preferred_element_type=f32)
        q_s[p] = jnp.where(diag, qp, 0.0)

    pro_compute(NPAIR, q_step)
    assert state["slab"] >= n_slab, state
    kv_start(k_hbm, 0, 0)
    kv_start(v_hbm, 0, 1)
    pro_idle(PRO[4])
    wm_cp(0, 2 * D, S_WMB, n=MR, nc=4 * D).wait()
    kv_start(k_hbm, 1, 2)
    kv_start(v_hbm, 1, 3)
    pro_compute(10, mod_step(5))
    pro_idle(PRO[5])
    assert state["piece"] == n_pro

    scale = DH ** -0.5

    def pair_step(p, acc):
        slot = lax.rem(p, AHEAD)
        ks = 2 * slot
        vs = ks + 1
        kv_wait(k_hbm, p, ks)
        q2 = q_s[p].astype(bf16)
        parts = []
        for k in range(T1):
            loop_piece(p, k)
            parts.append(jnp.dot(q2, big[ks, :, k * (W // T1):(k + 1) * (W // T1)], preferred_element_type=f32))
        s = jnp.concatenate(parts, axis=1) * scale
        m = jnp.max(s, axis=-1, keepdims=True)
        e = jnp.exp(s - m)
        l = jnp.sum(e, axis=-1, keepdims=True)
        e16 = e.astype(bf16)

        @pl.when(p + AHEAD < NPAIR)
        def _():
            kv_start(k_hbm, p + AHEAD, ks)

        ticks(N1, lambda i: loop_piece(p, T1 + i), D1)
        cur = lax.rem(p, 2)
        copy(wo_ref(cur), wo_ref(cur), S_WO + cur).wait()
        kv_wait(v_hbm, p, vs)
        o2 = jnp.zeros((8, PAIR), f32)
        for k in range(TPV):
            loop_piece(p, T1 + N1 + k)
            cs = slice(k * (W // TPV), (k + 1) * (W // TPV))
            o2 = o2 + lax.dot_general(e16[:, cs], big[vs, :, cs], (((1,), (1,)), ((), ())),
                                      preferred_element_type=f32)
        o2 = jnp.where(diag, o2 / l, 0.0).astype(bf16)
        for k, (r0, r1) in enumerate(((0, 128), (128, 256), (256, PAIR))):
            if 0 <= k - 1 < TWO:
                loop_piece(p, T1 + N1 + TPV + k - 1)
            acc = acc + jnp.dot(o2[:, r0:r1], big[cur, r0:r1, W:W + D], preferred_element_type=f32)

        @pl.when(p + AHEAD < NPAIR)
        def _():
            kv_start(v_hbm, p + AHEAD, vs)

        @pl.when(p + AHEAD == NPAIR - 1)
        def _():
            w1_cp.start(priority=1)
            for j in range(NW2):
                w2_cp(j).start(priority=1)

        ticks(jnp.where(p + 1 < NPAIR, n2, 0), lambda i: loop_piece(p, T1 + N1 + T2 + i), D2)
        return acc

    acc = lax.fori_loop(0, NPAIR, pair_step, jnp.zeros((8, D), f32))
    attn = jnp.sum(acc, axis=0, keepdims=True)

    ga, sb, cb, gb = (mod_s[:, i * D:(i + 1) * D] for i in range(2, 6))
    x1 = x32 + ga * attn

    h2 = (_layernorm(x1) * (1.0 + cb) + sb).astype(bf16)
    b1_cp.wait()
    b1 = b1_v[...].astype(f32)
    b1row = jnp.concatenate([b1[j:j + 1, :] for j in range(F // 128)], axis=1)
    copy(w1_v.at[pl.ds(0, w1_rows), :], w1_v.at[pl.ds(0, w1_rows), :], S_W1P).wait()
    w1_cp.wait()
    u = jnp.dot(h2, w1_v[...], preferred_element_type=f32) + b1row
    sp = jnp.log1p(jnp.exp(-jnp.abs(u))) + jnp.maximum(u, 0.0)
    act = (u * jnp.tanh(sp)).astype(bf16)
    copy(w2_ref(0).at[pl.ds(0, w2_rows), :], w2_ref(0).at[pl.ds(0, w2_rows), :], S_W2P).wait()
    y = jnp.zeros((8, D), f32)
    for j in range(NW2):
        w2_cp(j).wait()
        g, r0, r1 = w2_parts[j]
        if j == 0:
            r0 = 0
        y = y + jnp.dot(act[:, g * PAIR + r0:g * PAIR + r1], big[g, r0:r1, W + D:W + 2 * D],
                        preferred_element_type=f32)
    res = x1 + gb * y
    out_v[...] = res[0:1, :].astype(bf16)
    out_cp = copy(out_v, out_hbm, S_OUT)
    out_cp.start()
    out_cp.wait()


@jax.jit
def pallas_adaLN_cond__sliding_block_cached__dense_activation_mish__decode_kernel(
    A_x: jax.Array,
    A_k_cache: jax.Array,
    A_v_cache: jax.Array,
    A_wq: jax.Array,
    A_wo: jax.Array,
    B_x: jax.Array,
    B_w1: jax.Array,
    B_b1: jax.Array,
    B_w2: jax.Array,
    c: jax.Array,
    w_mod: jax.Array,
):
    del B_x
    SK = A_k_cache.shape[2]
    W = min(4096, max(256, SK // 4))
    kt = jnp.swapaxes(A_k_cache, 2, 3).reshape(H * DH, SK)
    vt = jnp.swapaxes(A_v_cache, 2, 3).reshape(H * DH, SK)
    x = A_x.reshape(1, D)
    b1 = B_b1.reshape(F // 128, 128)
    wm3 = w_mod.reshape(MG, MR, 6 * D)
    wq3 = A_wq.reshape(QG, QR, H * DH)
    wo3 = A_wo.reshape(NPAIR, PAIR, D)
    w23 = B_w2.reshape(F // PAIR, PAIR, D)

    any_spec = pl.BlockSpec(memory_space=pl.ANY)
    out = pl.pallas_call(
        functools.partial(_kernel, W=W, SK=SK),
        out_shape=jax.ShapeDtypeStruct((1, D), bf16),
        in_specs=[any_spec] * 10,
        out_specs=any_spec,
        scratch_shapes=[
            pltpu.VMEM((1, D), bf16),
            pltpu.VMEM((1, D), bf16),
            pltpu.VMEM((F // 128, 128), bf16),
            pltpu.VMEM((MG, MR, 6 * D), bf16),
            pltpu.VMEM((QG, QR, H * DH), bf16),
            pltpu.VMEM((NBUF, PAIR, W + 2 * D), bf16),
            pltpu.VMEM((D, F), bf16),
            pltpu.VMEM((NPAIR, 8, PAIR), f32),
            pltpu.VMEM((8, 6 * D), f32),
            pltpu.VMEM((1, D), bf16),
            pltpu.SemaphoreType.DMA((NSEM,)),
        ],
        compiler_params=pltpu.CompilerParams(
            vmem_limit_bytes=100 * 1024 * 1024,
            disable_bounds_checks=True,
            disable_semaphore_checks=True,
        ),
    )(x, c, b1, wm3, wq3, kt, vt, wo3, B_w1, w23)
    return out.reshape(1, 1, D)
```

```python
import functools

import jax
import jax.numpy as jnp
from jax import lax
import jax.experimental.pallas as pl
import jax.experimental.pallas.tpu as pltpu

D = 640
H = 32
DH = 192
F = 1536
PAIR = 2 * DH
NPAIR = H // 2
AHEAD = 2
NBUF = 2 * AHEAD
EPS = 1e-5

MG, MR = 10, 64
QG, QR = 8, 80
QC = 2048
NQC = H * DH // QC
KVO = (0, 1, 2, 3, 4, 5)
KVS = (1280, 640, 2176)

T1 = 8
TPV = 16
TWO = 2
T2 = TPV + TWO
N1 = 38
D1 = 82
D2 = 82
DP = 78
DP2 = 78
PPP = 96
PRO = (31, 39, 39, 39, 10, 28)
SL = 4
BULK0 = 10
NW2 = 5

f32 = jnp.float32
bf16 = jnp.bfloat16

S_C, S_X, S_B1, S_WMA, S_WMB, S_W1, S_W1P, S_W2P, S_OUT = range(9)
S_WO = 9
S_WQ = S_WO + 2
S_W2 = S_WQ + NQC
S_KV = S_W2 + NW2
NSEM = S_KV + NBUF


def _layernorm(x):
    m = jnp.mean(x, axis=-1, keepdims=True)
    xc = x - m
    v = jnp.mean(xc * xc, axis=-1, keepdims=True)
    return xc / jnp.sqrt(v + EPS)


def _kernel(x_hbm, c_hbm, b1_hbm, wmod_hbm, wq_hbm, k_hbm, v_hbm, wo_hbm, w1_hbm, w2_hbm,
            out_hbm,
            x_v, c_v, b1_v, wmod_v, wq_v, big, w1_v, q_s, mod_s, out_v, sem,
            *, W, SK):
    col0 = SK - W
    n2 = PPP - T1 - T2 - N1
    assert T1 % 2 == 0 and N1 % 2 == 0 and T2 % 2 == 0
    w2_pieces = T1 + N1 + T2
    w2_rows = 4 * w2_pieces

    def kv_ref(slot):
        return big.at[slot, :, pl.ds(0, W)]

    def wo_ref(slot):
        return big.at[slot, :, pl.ds(W, D)]

    def w2_ref(g):
        return big.at[g, :, pl.ds(W + D, D)]

    def mult(v, m):
        return v if isinstance(v, int) else pl.multiple_of(v, m)

    def copy(src, dst, s):
        return pltpu.make_async_copy(src, dst, sem.at[s])

    def ticks(n, tick, delay):
        def body(i, carry):
            tick(i)
            pl.delay(delay)
            return carry
        lax.fori_loop(0, n, body, 0)

    def wm_cp(i, c0, s, n=8, nc=2 * D):
        idx = (slice(None), pl.ds(mult(8 * i, 8), n), pl.ds(mult(c0, 128), nc))
        return copy(wmod_hbm.at[idx], wmod_v.at[idx], s)

    def wq_cp(j, i, n=8):
        idx = (slice(None), pl.ds(mult(8 * i, 8), n), pl.ds(mult(j * QC, 128), QC))
        return copy(wq_hbm.at[idx], wq_v.at[idx], S_WQ + j)

    def kv_cps(src, p, slot):
        rows = pl.ds(mult(p * PAIR, PAIR), PAIR)
        offs = [sum(KVS[:t]) for t in range(len(KVS))]
        return [copy(src.at[rows, pl.ds(col0 + offs[t], KVS[t])], big.at[slot, :, pl.ds(offs[t], KVS[t])],
                     S_KV + slot) for t in KVO if t < len(KVS)]

    def kv_start(src, p, slot):
        for d in kv_cps(src, p, slot):
            d.start(priority=1)

    def kv_wait(src, p, slot):
        copy(kv_ref(slot), kv_ref(slot), S_KV + slot).wait()

    n_wma, n_wq, n_wmb = MR // 8, NQC * (QR // 8), 2 * (MR // 8)
    n_slab = n_wma + n_wq + n_wmb

    def slab_start(i):
        if isinstance(i, int):
            if i < n_wma:
                wm_cp(i, 0, S_WMA).start(priority=1)
            elif i < n_wma + n_wq:
                wq_cp((i - n_wma) // (QR // 8), (i - n_wma) % (QR // 8)).start(priority=1)
            else:
                k = i - n_wma - n_wq
                wm_cp(k // 2, 2 * D + (k % 2) * 2 * D, S_WMB).start(priority=1)
            return

        @pl.when(i < n_wma + n_wq)
        def _():
            k = i - n_wma
            wq_cp(lax.div(k, QR // 8), lax.rem(k, QR // 8)).start(priority=1)

        @pl.when(jnp.logical_and(i >= n_wma + n_wq, i < n_slab))
        def _():
            k = i - n_wma - n_wq
            wm_cp(lax.div(k, 2), 2 * D + lax.rem(k, 2) * 2 * D, S_WMB).start(priority=1)

    def row_piece(src, dst, j, s):
        if isinstance(j, int):
            r = pl.ds((j // 2) * 8, 8)
            cs = pl.ds(0, PAIR) if j % 2 == 0 else pl.ds(PAIR, D - PAIR)
            copy(src.at[r, cs], dst.at[r, cs], s).start()
            return
        r = pl.ds(mult(lax.div(j, 2) * 8, 8), 8)

        @pl.when(lax.rem(j, 2) == 0)
        def _():
            copy(src.at[r, pl.ds(0, PAIR)], dst.at[r, pl.ds(0, PAIR)], s).start()

        @pl.when(lax.rem(j, 2) == 1)
        def _():
            copy(src.at[r, pl.ds(PAIR, D - PAIR)], dst.at[r, pl.ds(PAIR, D - PAIR)], s).start()

    def w1_piece(j):
        idx = (pl.ds(mult(lax.div(j, 4) * 8, 8), 8), pl.ds(mult(lax.rem(j, 4) * PAIR, 128), PAIR))
        copy(w1_hbm.at[idx], w1_v.at[idx], S_W1P).start()

    n_pro = sum(PRO) + 5 + NPAIR + 10
    w1_pieces = (n_pro - PPP) // 4 * 4
    w1_rows = 2 * w1_pieces

    def pro_piece(j):
        @pl.when(j < w1_pieces)
        def _():
            w1_piece(j)

        @pl.when(jnp.logical_and(j >= w1_pieces, j < w1_pieces + PPP))
        def _():
            row_piece(wo_hbm.at[0], wo_ref(0), j - w1_pieces, S_WO)

    def loop_piece(p, j):
        @pl.when(p + 1 < NPAIR)
        def _():
            nxt = lax.rem(p + 1, 2)
            row_piece(wo_hbm.at[p + 1], wo_ref(nxt), j, S_WO + nxt)

        @pl.when(p + 1 == NPAIR)
        def _():
            row_piece(w2_hbm.at[0], w2_ref(0), j, S_W2P)

    w1_cp = copy(w1_hbm.at[pl.ds(w1_rows, D - w1_rows), :], w1_v.at[pl.ds(w1_rows, D - w1_rows), :], S_W1)
    w2_parts = [(0, w2_rows, PAIR), (1, 0, PAIR), (2, 0, PAIR), (3, 0, 256), (3, 256, PAIR)]

    def w2_cp(j):
        g, r0, r1 = w2_parts[j]
        sl = pl.ds(r0, r1 - r0)
        return copy(w2_hbm.at[g, sl, :], w2_ref(g).at[sl, :], S_W2 + j)

    x_cp = copy(x_hbm, x_v, S_X)
    c_cp = copy(c_hbm, c_v, S_C)
    b1_cp = copy(b1_hbm, b1_v, S_B1)
    slab_start(0)
    c_cp.start()
    x_cp.start()
    for i in range(1, BULK0):
        slab_start(i)
    b1_cp.start()

    state = {"piece": 0, "slab": BULK0}

    def pro_idle(n):
        j0, i0 = state["piece"], state["slab"]

        def tick(i):
            pro_piece(j0 + i)

            if i0 < n_slab:
                @pl.when(lax.rem(i, SL) == 0)
                def _():
                    slab_start(i0 + lax.div(i, SL))

        ticks(n, tick, DP if i0 < n_slab else DP2)
        state["piece"] += n
        state["slab"] += -(-n // SL)

    def pro_compute(n, step):
        j0, i0 = state["piece"], state["slab"]

        def body(i, carry):
            pro_piece(j0 + i)

            if i0 < n_slab:
                @pl.when(lax.rem(i, 2) == 0)
                def _():
                    slab_start(i0 + lax.div(i, 2))

            step(i)
            return carry

        lax.fori_loop(0, n, body, 0)
        state["piece"] += n
        state["slab"] += -(-n // 2)

    pro_idle(PRO[0])
    c_cp.wait()
    x_cp.wait()
    c32 = c_v[...].astype(f32)
    sc = c32 * jax.nn.sigmoid(c32)
    sc8 = jnp.broadcast_to(sc, (8, D)).astype(bf16)
    x32 = x_v[...].astype(f32)
    xn = _layernorm(x32)

    def mod_step(first):
        def step(i):
            cs = pl.ds(pl.multiple_of((first + i) * 256, 256), 256)
            mod_s[:, cs] = jnp.dot(sc8, wmod_v[:, :, cs].reshape(D, 256), preferred_element_type=f32)
        return step

    wm_cp(0, 0, S_WMA, n=MR).wait()
    pro_compute(5, mod_step(0))
    h = xn * (1.0 + mod_s[:, D:2 * D]) + mod_s[:, 0:D]
    h8 = h.astype(bf16)

    row = lax.broadcasted_iota(jnp.int32, (8, PAIR), 0)
    lane = lax.broadcasted_iota(jnp.int32, (8, PAIR), 1)
    diag = (row == jnp.where(lane >= DH, 1, 0))

    for j in range(3):
        pro_idle(PRO[1 + j])
    assert state["slab"] >= n_wma + n_wq, state
    for j in range(NQC):
        wq_cp(j, 0, n=QR).wait()

    def q_step(p):
        cs = pl.ds(pl.multiple_of(p * PAIR, 128), PAIR)
        qp = jnp.dot(h8, wq_v[:, :, cs].reshape(D, PAIR), preferred_element_type=f32)
        q_s[p] = jnp.where(diag, qp, 0.0)

    pro_compute(NPAIR, q_step)
    assert state["slab"] >= n_slab, state
    kv_start(k_hbm, 0, 0)
    kv_start(v_hbm, 0, 1)
    pro_idle(PRO[4])
    wm_cp(0, 2 * D, S_WMB, n=MR, nc=4 * D).wait()
    kv_start(k_hbm, 1, 2)
    kv_start(v_hbm, 1, 3)
    pro_compute(10, mod_step(5))
    pro_idle(PRO[5])
    assert state["piece"] == n_pro

    scale = DH ** -0.5

    def pair_step(p, acc):
        slot = lax.rem(p, AHEAD)
        ks = 2 * slot
        vs = ks + 1
        kv_wait(k_hbm, p, ks)
        q2 = q_s[p].astype(bf16)
        parts = []
        for k in range(T1):
            loop_piece(p, k)
            parts.append(jnp.dot(q2, big[ks, :, k * (W // T1):(k + 1) * (W // T1)], preferred_element_type=f32))
        s = jnp.concatenate(parts, axis=1) * scale
        m = jnp.max(s, axis=-1, keepdims=True)
        e = jnp.exp(s - m)
        l = jnp.sum(e, axis=-1, keepdims=True)
        e16 = e.astype(bf16)

        @pl.when(p + AHEAD < NPAIR)
        def _():
            kv_start(k_hbm, p + AHEAD, ks)

        ticks(N1, lambda i: loop_piece(p, T1 + i), D1)
        cur = lax.rem(p, 2)
        copy(wo_ref(cur), wo_ref(cur), S_WO + cur).wait()
        kv_wait(v_hbm, p, vs)
        o2 = jnp.zeros((8, PAIR), f32)
        for k in range(TPV):
            loop_piece(p, T1 + N1 + k)
            cs = slice(k * (W // TPV), (k + 1) * (W // TPV))
            o2 = o2 + lax.dot_general(e16[:, cs], big[vs, :, cs], (((1,), (1,)), ((), ())),
                                      preferred_element_type=f32)
        o2 = jnp.where(diag, o2 / l, 0.0).astype(bf16)
        for k, (r0, r1) in enumerate(((0, 128), (128, 256), (256, PAIR))):
            if 0 <= k - 1 < TWO:
                loop_piece(p, T1 + N1 + TPV + k - 1)
            acc = acc + jnp.dot(o2[:, r0:r1], big[cur, r0:r1, W:W + D], preferred_element_type=f32)

        @pl.when(p + AHEAD < NPAIR)
        def _():
            kv_start(v_hbm, p + AHEAD, vs)

        @pl.when(p + AHEAD == NPAIR - 1)
        def _():
            w1_cp.start(priority=1)
            for j in range(NW2):
                w2_cp(j).start(priority=1)

        ticks(jnp.where(p + 1 < NPAIR, n2, 0), lambda i: loop_piece(p, T1 + N1 + T2 + i), D2)
        return acc

    acc = lax.fori_loop(0, NPAIR, pair_step, jnp.zeros((8, D), f32))
    attn = jnp.sum(acc, axis=0, keepdims=True)

    ga, sb, cb, gb = (mod_s[:, i * D:(i + 1) * D] for i in range(2, 6))
    x1 = x32 + ga * attn

    h2 = (_layernorm(x1) * (1.0 + cb) + sb).astype(bf16)
    b1_cp.wait()
    b1 = b1_v[...].astype(f32)
    b1row = jnp.concatenate([b1[j:j + 1, :] for j in range(F // 128)], axis=1)
    copy(w1_v.at[pl.ds(0, w1_rows), :], w1_v.at[pl.ds(0, w1_rows), :], S_W1P).wait()
    w1_cp.wait()
    u = jnp.dot(h2, w1_v[...], preferred_element_type=f32) + b1row
    sp = jnp.log1p(jnp.exp(-jnp.abs(u))) + jnp.maximum(u, 0.0)
    act = (u * jnp.tanh(sp)).astype(bf16)
    copy(w2_ref(0).at[pl.ds(0, w2_rows), :], w2_ref(0).at[pl.ds(0, w2_rows), :], S_W2P).wait()
    y = jnp.zeros((8, D), f32)
    for j in range(NW2):
        w2_cp(j).wait()
        g, r0, r1 = w2_parts[j]
        if j == 0:
            r0 = 0
        y = y + jnp.dot(act[:, g * PAIR + r0:g * PAIR + r1], big[g, r0:r1, W + D:W + 2 * D],
                        preferred_element_type=f32)
    res = x1 + gb * y
    out_v[...] = res[0:1, :].astype(bf16)
    out_cp = copy(out_v, out_hbm, S_OUT)
    out_cp.start()
    out_cp.wait()


@jax.jit
def pallas_adaLN_cond__sliding_block_cached__dense_activation_mish__decode_kernel(
    A_x: jax.Array,
    A_k_cache: jax.Array,
    A_v_cache: jax.Array,
    A_wq: jax.Array,
    A_wo: jax.Array,
    B_x: jax.Array,
    B_w1: jax.Array,
    B_b1: jax.Array,
    B_w2: jax.Array,
    c: jax.Array,
    w_mod: jax.Array,
):
    del B_x
    SK = A_k_cache.shape[2]
    W = min(4096, max(256, SK // 4))
    kt = jnp.swapaxes(A_k_cache, 2, 3).reshape(H * DH, SK)
    vt = jnp.swapaxes(A_v_cache, 2, 3).reshape(H * DH, SK)
    x = A_x.reshape(1, D)
    b1 = B_b1.reshape(F // 128, 128)
    wm3 = w_mod.reshape(MG, MR, 6 * D)
    wq3 = A_wq.reshape(QG, QR, H * DH)
    wo3 = A_wo.reshape(NPAIR, PAIR, D)
    w23 = B_w2.reshape(F // PAIR, PAIR, D)

    any_spec = pl.BlockSpec(memory_space=pl.ANY)
    out = pl.pallas_call(
        functools.partial(_kernel, W=W, SK=SK),
        out_shape=jax.ShapeDtypeStruct((1, D), bf16),
        in_specs=[any_spec] * 10,
        out_specs=any_spec,
        scratch_shapes=[
            pltpu.VMEM((1, D), bf16),
            pltpu.VMEM((1, D), bf16),
            pltpu.VMEM((F // 128, 128), bf16),
            pltpu.VMEM((MG, MR, 6 * D), bf16),
            pltpu.VMEM((QG, QR, H * DH), bf16),
            pltpu.VMEM((NBUF, PAIR, W + 2 * D), bf16),
            pltpu.VMEM((D, F), bf16),
            pltpu.VMEM((NPAIR, 8, PAIR), f32),
            pltpu.VMEM((8, 6 * D), f32),
            pltpu.VMEM((1, D), bf16),
            pltpu.SemaphoreType.DMA((NSEM,)),
        ],
        compiler_params=pltpu.CompilerParams(
            vmem_limit_bytes=100 * 1024 * 1024,
            disable_bounds_checks=True,
            disable_semaphore_checks=True,
        ),
    )(x, c, b1, wm3, wq3, kt, vt, wo3, B_w1, w23)
    return out.reshape(1, 1, D)
```

```python
import functools

import jax
import jax.numpy as jnp
from jax import lax
import jax.experimental.pallas as pl
import jax.experimental.pallas.tpu as pltpu

D = 640
H = 32
DH = 192
F = 1536
PAIR = 2 * DH
NPAIR = H // 2
AHEAD = 2
NBUF = 2 * AHEAD
EPS = 1e-5

MG, MR = 10, 64
QG, QR = 8, 80
QS = (2048, 2048, 2048)
NQC = len(QS)
KVO = (0, 1, 2, 3, 4, 5)
KVS = (1280, 640, 2176)

T1 = 8
TPV = 16
TWO = 2
T2 = TPV + TWO
N1 = 38
D1 = 62
D2 = 62
DP = 61
DP2 = 62
PPP = 96
PRO = (31, 39, 39, 39, 10, 28)
SL = 4
BULK0 = 10
NW2 = 5

f32 = jnp.float32
bf16 = jnp.bfloat16

S_C, S_X, S_B1, S_WMA, S_WMB, S_W1, S_W1P, S_W2P, S_OUT = range(9)
S_WO = 9
S_WQ = S_WO + 2
S_W2 = S_WQ + NQC
S_KV = S_W2 + NW2
NSEM = S_KV + NBUF


def _layernorm(x):
    m = jnp.mean(x, axis=-1, keepdims=True)
    xc = x - m
    v = jnp.mean(xc * xc, axis=-1, keepdims=True)
    return xc / jnp.sqrt(v + EPS)


def _kernel(x_hbm, c_hbm, b1_hbm, wmod_hbm, wq_hbm, k_hbm, v_hbm, wo_hbm, w1_hbm, w2_hbm,
            out_hbm,
            x_v, c_v, b1_v, wmod_v, wq_v, big, w1_v, q_s, mod_s, out_v, pace_s, sem,
            *, W, SK):
    col0 = SK - W
    n2 = PPP - T1 - T2 - N1
    assert T1 % 2 == 0 and N1 % 2 == 0 and T2 % 2 == 0
    w2_pieces = T1 + N1 + T2
    w2_rows = 4 * w2_pieces

    def kv_ref(slot):
        return big.at[slot, :, pl.ds(0, W)]

    def wo_ref(slot):
        return big.at[slot, :, pl.ds(W, D)]

    def w2_ref(g):
        return big.at[g, :, pl.ds(W + D, D)]

    def mult(v, m):
        return v if isinstance(v, int) else pl.multiple_of(v, m)

    def copy(src, dst, s):
        return pltpu.make_async_copy(src, dst, sem.at[s])

    def ticks(n, tick, delay):
        def body(i, v):
            tick(i)
            for k in range(delay):
                v = v * 0.5 if k % 2 == 0 else v + 0.25
            return v
        pace_s[...] = lax.fori_loop(0, n, body, pace_s[...])

    def wm_cp(i, c0, s, n=8, nc=2 * D):
        idx = (slice(None), pl.ds(mult(8 * i, 8), n), pl.ds(mult(c0, 128), nc))
        return copy(wmod_hbm.at[idx], wmod_v.at[idx], s)

    def wq_cp(j, i, n=8):
        idx = (slice(None), pl.ds(mult(8 * i, 8), n), pl.ds(sum(QS[:j]), QS[j]))
        return copy(wq_hbm.at[idx], wq_v.at[idx], S_WQ + j)

    def kv_cps(src, p, slot):
        rows = pl.ds(mult(p * PAIR, PAIR), PAIR)
        offs = [sum(KVS[:t]) for t in range(len(KVS))]
        return [copy(src.at[rows, pl.ds(col0 + offs[t], KVS[t])], big.at[slot, :, pl.ds(offs[t], KVS[t])],
                     S_KV + slot) for t in KVO if t < len(KVS)]

    def kv_start(src, p, slot):
        for d in kv_cps(src, p, slot):
            d.start(priority=1)

    def kv_wait(src, p, slot):
        copy(kv_ref(slot), kv_ref(slot), S_KV + slot).wait()

    n_wma, n_wq, n_wmb = MR // 8, NQC * (QR // 8), 2 * (MR // 8)
    n_slab = n_wma + n_wq + n_wmb

    def slab_start(i):
        if isinstance(i, int):
            if i < n_wma:
                wm_cp(i, 0, S_WMA).start(priority=1)
            elif i < n_wma + n_wq:
                wq_cp((i - n_wma) // (QR // 8), (i - n_wma) % (QR // 8)).start(priority=1)
            else:
                k = i - n_wma - n_wq
                wm_cp(k // 2, 2 * D + (k % 2) * 2 * D, S_WMB).start(priority=1)
            return

        for j in range(NQC):
            lo = n_wma + j * (QR // 8)

            @pl.when(jnp.logical_and(i >= lo, i < lo + QR // 8))
            def _():
                wq_cp(j, i - lo).start(priority=1)

        @pl.when(jnp.logical_and(i >= n_wma + n_wq, i < n_slab))
        def _():
            k = i - n_wma - n_wq
            wm_cp(lax.div(k, 2), 2 * D + lax.rem(k, 2) * 2 * D, S_WMB).start(priority=1)

    def row_piece(src, dst, j, s):
        if isinstance(j, int):
            r = pl.ds((j // 2) * 8, 8)
            cs = pl.ds(0, PAIR) if j % 2 == 0 else pl.ds(PAIR, D - PAIR)
            copy(src.at[r, cs], dst.at[r, cs], s).start()
            return
        r = pl.ds(mult(lax.div(j, 2) * 8, 8), 8)

        @pl.when(lax.rem(j, 2) == 0)
        def _():
            copy(src.at[r, pl.ds(0, PAIR)], dst.at[r, pl.ds(0, PAIR)], s).start()

        @pl.when(lax.rem(j, 2) == 1)
        def _():
            copy(src.at[r, pl.ds(PAIR, D - PAIR)], dst.at[r, pl.ds(PAIR, D - PAIR)], s).start()

    def w1_piece(j):
        idx = (pl.ds(mult(lax.div(j, 4) * 8, 8), 8), pl.ds(mult(lax.rem(j, 4) * PAIR, 128), PAIR))
        copy(w1_hbm.at[idx], w1_v.at[idx], S_W1P).start()

    n_pro = sum(PRO) + 5 + NPAIR + 10
    w1_pieces = (n_pro - PPP) // 4 * 4
    w1_rows = 2 * w1_pieces

    def pro_piece(j):
        @pl.when(j < w1_pieces)
        def _():
            w1_piece(j)

        @pl.when(jnp.logical_and(j >= w1_pieces, j < w1_pieces + PPP))
        def _():
            row_piece(wo_hbm.at[0], wo_ref(0), j - w1_pieces, S_WO)

    def loop_piece(p, j):
        @pl.when(p + 1 < NPAIR)
        def _():
            nxt = lax.rem(p + 1, 2)
            row_piece(wo_hbm.at[p + 1], wo_ref(nxt), j, S_WO + nxt)

        @pl.when(p + 1 == NPAIR)
        def _():
            row_piece(w2_hbm.at[0], w2_ref(0), j, S_W2P)

    w1_cp = copy(w1_hbm.at[pl.ds(w1_rows, D - w1_rows), :], w1_v.at[pl.ds(w1_rows, D - w1_rows), :], S_W1)
    w2_parts = [(0, w2_rows, PAIR), (1, 0, PAIR), (2, 0, PAIR), (3, 0, 256), (3, 256, PAIR)]

    def w2_cp(j):
        g, r0, r1 = w2_parts[j]
        sl = pl.ds(r0, r1 - r0)
        return copy(w2_hbm.at[g, sl, :], w2_ref(g).at[sl, :], S_W2 + j)

    x_cp = copy(x_hbm, x_v, S_X)
    c_cp = copy(c_hbm, c_v, S_C)
    b1_cp = copy(b1_hbm, b1_v, S_B1)
    slab_start(0)
    c_cp.start()
    x_cp.start()
    for i in range(1, BULK0):
        slab_start(i)
    b1_cp.start()
    pace_s[...] = lax.broadcasted_iota(jnp.int32, (8, 128), 1).astype(f32)

    state = {"piece": 0, "slab": BULK0}

    def pro_idle(n):
        j0, i0 = state["piece"], state["slab"]

        def tick(i):
            pro_piece(j0 + i)

            if i0 < n_slab:
                @pl.when(lax.rem(i, SL) == 0)
                def _():
                    slab_start(i0 + lax.div(i, SL))

        ticks(n, tick, DP if i0 < n_slab else DP2)
        state["piece"] += n
        state["slab"] += -(-n // SL)

    def pro_compute(n, step):
        j0, i0 = state["piece"], state["slab"]

        def body(i, carry):
            pro_piece(j0 + i)

            if i0 < n_slab:
                @pl.when(lax.rem(i, 2) == 0)
                def _():
                    slab_start(i0 + lax.div(i, 2))

            step(i)
            return carry

        lax.fori_loop(0, n, body, 0)
        state["piece"] += n
        state["slab"] += -(-n // 2)

    pro_idle(PRO[0])
    c_cp.wait()
    x_cp.wait()
    c32 = c_v[...].astype(f32)
    sc = c32 * jax.nn.sigmoid(c32)
    sc8 = jnp.broadcast_to(sc, (8, D)).astype(bf16)
    x32 = x_v[...].astype(f32)
    xn = _layernorm(x32)

    def mod_step(first):
        def step(i):
            cs = pl.ds(pl.multiple_of((first + i) * 256, 256), 256)
            mod_s[:, cs] = jnp.dot(sc8, wmod_v[:, :, cs].reshape(D, 256), preferred_element_type=f32)
        return step

    wm_cp(0, 0, S_WMA, n=MR).wait()
    pro_compute(5, mod_step(0))
    h = xn * (1.0 + mod_s[:, D:2 * D]) + mod_s[:, 0:D]
    h8 = h.astype(bf16)

    row = lax.broadcasted_iota(jnp.int32, (8, PAIR), 0)
    lane = lax.broadcasted_iota(jnp.int32, (8, PAIR), 1)
    diag = (row == jnp.where(lane >= DH, 1, 0))

    for j in range(3):
        pro_idle(PRO[1 + j])
    assert state["slab"] >= n_wma + n_wq, state
    for j in range(NQC):
        wq_cp(j, 0, n=QR).wait()

    def q_step(p):
        cs = pl.ds(pl.multiple_of(p * PAIR, 128), PAIR)
        qp = jnp.dot(h8, wq_v[:, :, cs].reshape(D, PAIR), preferred_element_type=f32)
        q_s[p] = jnp.where(diag, qp, 0.0)

    pro_compute(NPAIR, q_step)
    assert state["slab"] >= n_slab, state
    kv_start(k_hbm, 0, 0)
    kv_start(v_hbm, 0, 1)
    pro_idle(PRO[4])
    wm_cp(0, 2 * D, S_WMB, n=MR, nc=4 * D).wait()
    kv_start(k_hbm, 1, 2)
    kv_start(v_hbm, 1, 3)
    pro_compute(10, mod_step(5))
    pro_idle(PRO[5])
    assert state["piece"] == n_pro

    scale = DH ** -0.5

    def pair_step(p, acc):
        slot = lax.rem(p, AHEAD)
        ks = 2 * slot
        vs = ks + 1
        kv_wait(k_hbm, p, ks)
        q2 = q_s[p].astype(bf16)
        parts = []
        for k in range(T1):
            loop_piece(p, k)
            parts.append(jnp.dot(q2, big[ks, :, k * (W // T1):(k + 1) * (W // T1)], preferred_element_type=f32))
        s = jnp.concatenate(parts, axis=1) * scale
        m = jnp.max(s, axis=-1, keepdims=True)
        e = jnp.exp(s - m)
        l = jnp.sum(e, axis=-1, keepdims=True)
        e16 = e.astype(bf16)

        @pl.when(p + AHEAD < NPAIR)
        def _():
            kv_start(k_hbm, p + AHEAD, ks)

        ticks(N1, lambda i: loop_piece(p, T1 + i), D1)
        cur = lax.rem(p, 2)
        copy(wo_ref(cur), wo_ref(cur), S_WO + cur).wait()
        kv_wait(v_hbm, p, vs)
        o2 = jnp.zeros((8, PAIR), f32)
        for k in range(TPV):
            loop_piece(p, T1 + N1 + k)
            cs = slice(k * (W // TPV), (k + 1) * (W // TPV))
            o2 = o2 + lax.dot_general(e16[:, cs], big[vs, :, cs], (((1,), (1,)), ((), ())),
                                      preferred_element_type=f32)
        o2 = jnp.where(diag, o2 / l, 0.0).astype(bf16)
        for k, (r0, r1) in enumerate(((0, 128), (128, 256), (256, PAIR))):
            if 0 <= k - 1 < TWO:
                loop_piece(p, T1 + N1 + TPV + k - 1)
            acc = acc + jnp.dot(o2[:, r0:r1], big[cur, r0:r1, W:W + D], preferred_element_type=f32)

        @pl.when(p + AHEAD < NPAIR)
        def _():
            kv_start(v_hbm, p + AHEAD, vs)

        @pl.when(p + AHEAD == NPAIR - 1)
        def _():
            w1_cp.start(priority=1)
            for j in range(NW2):
                w2_cp(j).start(priority=1)

        ticks(jnp.where(p + 1 < NPAIR, n2, 0), lambda i: loop_piece(p, T1 + N1 + T2 + i), D2)
        return acc

    acc = lax.fori_loop(0, NPAIR, pair_step, jnp.zeros((8, D), f32))
    attn = jnp.sum(acc, axis=0, keepdims=True)

    ga, sb, cb, gb = (mod_s[:, i * D:(i + 1) * D] for i in range(2, 6))
    x1 = x32 + ga * attn

    h2 = (_layernorm(x1) * (1.0 + cb) + sb).astype(bf16)
    b1_cp.wait()
    b1 = b1_v[...].astype(f32)
    b1row = jnp.concatenate([b1[j:j + 1, :] for j in range(F // 128)], axis=1)
    copy(w1_v.at[pl.ds(0, w1_rows), :], w1_v.at[pl.ds(0, w1_rows), :], S_W1P).wait()
    w1_cp.wait()
    u = jnp.dot(h2, w1_v[...], preferred_element_type=f32) + b1row
    sp = jnp.log1p(jnp.exp(-jnp.abs(u))) + jnp.maximum(u, 0.0)
    act = (u * jnp.tanh(sp)).astype(bf16)
    copy(w2_ref(0).at[pl.ds(0, w2_rows), :], w2_ref(0).at[pl.ds(0, w2_rows), :], S_W2P).wait()
    y = jnp.zeros((8, D), f32)
    for j in range(NW2):
        w2_cp(j).wait()
        g, r0, r1 = w2_parts[j]
        if j == 0:
            r0 = 0
        y = y + jnp.dot(act[:, g * PAIR + r0:g * PAIR + r1], big[g, r0:r1, W + D:W + 2 * D],
                        preferred_element_type=f32)
    res = x1 + gb * y
    out_v[...] = res[0:1, :].astype(bf16)
    out_cp = copy(out_v, out_hbm, S_OUT)
    out_cp.start()
    out_cp.wait()


@jax.jit
def pallas_adaLN_cond__sliding_block_cached__dense_activation_mish__decode_kernel(
    A_x: jax.Array,
    A_k_cache: jax.Array,
    A_v_cache: jax.Array,
    A_wq: jax.Array,
    A_wo: jax.Array,
    B_x: jax.Array,
    B_w1: jax.Array,
    B_b1: jax.Array,
    B_w2: jax.Array,
    c: jax.Array,
    w_mod: jax.Array,
):
    del B_x
    SK = A_k_cache.shape[2]
    W = min(4096, max(256, SK // 4))
    kt = jnp.swapaxes(A_k_cache, 2, 3).reshape(H * DH, SK)
    vt = jnp.swapaxes(A_v_cache, 2, 3).reshape(H * DH, SK)
    x = A_x.reshape(1, D)
    b1 = B_b1.reshape(F // 128, 128)
    wm3 = w_mod.reshape(MG, MR, 6 * D)
    wq3 = A_wq.reshape(QG, QR, H * DH)
    wo3 = A_wo.reshape(NPAIR, PAIR, D)
    w23 = B_w2.reshape(F // PAIR, PAIR, D)

    any_spec = pl.BlockSpec(memory_space=pl.ANY)
    out = pl.pallas_call(
        functools.partial(_kernel, W=W, SK=SK),
        out_shape=jax.ShapeDtypeStruct((1, D), bf16),
        in_specs=[any_spec] * 10,
        out_specs=any_spec,
        scratch_shapes=[
            pltpu.VMEM((1, D), bf16),
            pltpu.VMEM((1, D), bf16),
            pltpu.VMEM((F // 128, 128), bf16),
            pltpu.VMEM((MG, MR, 6 * D), bf16),
            pltpu.VMEM((QG, QR, H * DH), bf16),
            pltpu.VMEM((NBUF, PAIR, W + 2 * D), bf16),
            pltpu.VMEM((D, F), bf16),
            pltpu.VMEM((NPAIR, 8, PAIR), f32),
            pltpu.VMEM((8, 6 * D), f32),
            pltpu.VMEM((1, D), bf16),
            pltpu.VMEM((8, 128), f32),
            pltpu.SemaphoreType.DMA((NSEM,)),
        ],
        compiler_params=pltpu.CompilerParams(
            vmem_limit_bytes=100 * 1024 * 1024,
            disable_bounds_checks=True,
            disable_semaphore_checks=True,
        ),
    )(x, c, b1, wm3, wq3, kt, vt, wo3, B_w1, w23)
    return out.reshape(1, 1, D)
```

```python
import functools

import jax
import jax.numpy as jnp
from jax import lax
import jax.experimental.pallas as pl
import jax.experimental.pallas.tpu as pltpu

D = 640
H = 32
DH = 192
F = 1536
PAIR = 2 * DH
NPAIR = H // 2
AHEAD = 2
NBUF = 2 * AHEAD
EPS = 1e-5

G, GR = 10, 64
NRT = GR // 8
QC = 2048
NQC = H * DH // QC
KV_COLS = (1280, 640, 2176)
N_WMA, N_WQ, N_WMB = NRT, NRT * NQC, 2 * NRT
N_SLAB = N_WMA + N_WQ + N_WMB
SLABS_UP_FRONT = 10
SLAB_EVERY = 5

PPP = 96
T_QK, T_PV, T_WO = 8, 16, 2
N1 = 38
N2 = PPP - T_QK - T_PV - T_WO - N1
PRO = (33, 39, 39, 39, 10, 30)
PACE = 62
PACE_SLAB = 61
N_PRO = sum(PRO) + 5 + NPAIR + 10
W1_PIECES = (N_PRO - PPP) // 4 * 4
W1_ROWS = 2 * W1_PIECES
W2_ROWS = 4 * (T_QK + N1 + T_PV + T_WO)
W2_PARTS = ((0, W2_ROWS, PAIR), (1, 0, PAIR), (2, 0, PAIR), (3, 0, 256), (3, 256, PAIR))

f32 = jnp.float32
bf16 = jnp.bfloat16

S_C, S_X, S_B1, S_WMA, S_WMB, S_WQ, S_W1, S_W1P, S_W2P, S_OUT = range(10)
S_WO = 10
S_W2 = S_WO + 2
S_KV = S_W2 + len(W2_PARTS)
NSEM = S_KV + NBUF


def _layernorm(x):
    m = jnp.mean(x, axis=-1, keepdims=True)
    xc = x - m
    v = jnp.mean(xc * xc, axis=-1, keepdims=True)
    return xc / jnp.sqrt(v + EPS)


def _kernel(x_hbm, c_hbm, b1_hbm, wmod_hbm, wq_hbm, k_hbm, v_hbm, wo_hbm, w1_hbm, w2_hbm,
            out_hbm,
            x_v, c_v, b1_v, wmod_v, wq_v, big, w1_v, q_s, mod_s, out_v, pace_s, sem,
            *, W, SK):
    col0 = SK - W

    def kv_ref(slot):
        return big.at[slot, :, pl.ds(0, W)]

    def wo_ref(slot):
        return big.at[slot, :, pl.ds(W, D)]

    def w2_ref(g):
        return big.at[g, :, pl.ds(W + D, D)]

    def mult(v, m):
        return v if isinstance(v, int) else pl.multiple_of(v, m)

    def copy(src, dst, s):
        return pltpu.make_async_copy(src, dst, sem.at[s])

    def wait_filled(buf, s):
        copy(buf, buf, s).wait()

    def ticks(n, tick, pace):
        def body(i, v):
            tick(i)
            for k in range(pace):
                v = v * 0.5 if k % 2 == 0 else v + 0.25
            return v
        pace_s[...] = lax.fori_loop(0, n, body, pace_s[...])

    def slab(src, dst, rt, c0, nc, s):
        idx = (slice(None), pl.ds(mult(8 * rt, 8), 8), pl.ds(mult(c0, 128), nc))
        copy(src.at[idx], dst.at[idx], s).start(priority=1)

    def slab_start(i):
        if isinstance(i, int):
            if i < N_WMA:
                slab(wmod_hbm, wmod_v, i, 0, 2 * D, S_WMA)
            else:
                slab(wq_hbm, wq_v, (i - N_WMA) // NQC, (i - N_WMA) % NQC * QC, QC, S_WQ)
            return

        @pl.when(i < N_WMA + N_WQ)
        def _():
            k = i - N_WMA
            slab(wq_hbm, wq_v, lax.div(k, NQC), lax.rem(k, NQC) * QC, QC, S_WQ)

        @pl.when(jnp.logical_and(i >= N_WMA + N_WQ, i < N_SLAB))
        def _():
            k = i - N_WMA - N_WQ
            slab(wmod_hbm, wmod_v, lax.div(k, 2), (1 + lax.rem(k, 2)) * 2 * D, 2 * D, S_WMB)

    def kv_start(src, p, slot):
        rows = pl.ds(mult(p * PAIR, PAIR), PAIR)
        c0 = 0
        for nc in KV_COLS:
            copy(src.at[rows, pl.ds(col0 + c0, nc)], big.at[slot, :, pl.ds(c0, nc)], S_KV + slot).start(priority=1)
            c0 += nc

    w1_rest = pl.ds(W1_ROWS, D - W1_ROWS)
    w1_cp = copy(w1_hbm.at[w1_rest, :], w1_v.at[w1_rest, :], S_W1)

    def w2_cp(j):
        g, r0, r1 = W2_PARTS[j]
        rows = pl.ds(r0, r1 - r0)
        return copy(w2_hbm.at[g, rows, :], w2_ref(g).at[rows, :], S_W2 + j)

    def row_piece(src, dst, j, s):
        parts = (pl.ds(0, PAIR), pl.ds(PAIR, D - PAIR))
        if isinstance(j, int):
            r = pl.ds(j // 2 * 8, 8)
            copy(src.at[r, parts[j % 2]], dst.at[r, parts[j % 2]], s).start()
            return
        r = pl.ds(pl.multiple_of(lax.div(j, 2) * 8, 8), 8)
        for half in range(2):
            @pl.when(lax.rem(j, 2) == half)
            def _():
                copy(src.at[r, parts[half]], dst.at[r, parts[half]], s).start()

    def pro_piece(j):
        @pl.when(j < W1_PIECES)
        def _():
            idx = (pl.ds(pl.multiple_of(lax.div(j, 4) * 8, 8), 8),
                   pl.ds(pl.multiple_of(lax.rem(j, 4) * PAIR, 128), PAIR))
            copy(w1_hbm.at[idx], w1_v.at[idx], S_W1P).start()

        @pl.when(jnp.logical_and(j >= W1_PIECES, j < W1_PIECES + PPP))
        def _():
            row_piece(wo_hbm.at[0], wo_ref(0), j - W1_PIECES, S_WO)

    def loop_piece(p, j):
        @pl.when(p + 1 < NPAIR)
        def _():
            nxt = lax.rem(p + 1, 2)
            row_piece(wo_hbm.at[p + 1], wo_ref(nxt), j, S_WO + nxt)

        @pl.when(p + 1 == NPAIR)
        def _():
            row_piece(w2_hbm.at[0], w2_ref(0), j, S_W2P)

    x_cp = copy(x_hbm, x_v, S_X)
    c_cp = copy(c_hbm, c_v, S_C)
    b1_cp = copy(b1_hbm, b1_v, S_B1)
    slab_start(0)
    c_cp.start()
    x_cp.start()
    for i in range(1, SLABS_UP_FRONT):
        slab_start(i)
    b1_cp.start()
    pace_s[...] = lax.broadcasted_iota(jnp.int32, (8, 128), 1).astype(f32)

    pos = {"piece": 0, "slab": SLABS_UP_FRONT}

    def pro_tick(every):
        j0, i0 = pos["piece"], pos["slab"]

        def tick(i):
            pro_piece(j0 + i)
            if i0 < N_SLAB:
                @pl.when(lax.rem(i, every) == 0)
                def _():
                    slab_start(i0 + lax.div(i, every))
        return tick

    def pro_idle(n):
        ticks(n, pro_tick(SLAB_EVERY), PACE_SLAB if pos["slab"] < N_SLAB else PACE)
        pos["piece"] += n
        pos["slab"] += -(-n // SLAB_EVERY)

    def pro_compute(n, step):
        tick = pro_tick(2)

        def body(i, carry):
            tick(i)
            step(i)
            return carry
        lax.fori_loop(0, n, body, 0)
        pos["piece"] += n
        pos["slab"] += -(-n // 2)

    pro_idle(PRO[0])
    c_cp.wait()
    x_cp.wait()
    c32 = c_v[...].astype(f32)
    sc8 = jnp.broadcast_to(c32 * jax.nn.sigmoid(c32), (8, D)).astype(bf16)
    x32 = x_v[...].astype(f32)
    xn = _layernorm(x32)

    def mod_step(first):
        def step(i):
            cs = pl.ds(pl.multiple_of((first + i) * 256, 256), 256)
            mod_s[:, cs] = jnp.dot(sc8, wmod_v[:, :, cs].reshape(D, 256), preferred_element_type=f32)
        return step

    wait_filled(wmod_v.at[:, :, pl.ds(0, 2 * D)], S_WMA)
    pro_compute(5, mod_step(0))
    h8 = (xn * (1.0 + mod_s[:, D:2 * D]) + mod_s[:, 0:D]).astype(bf16)

    row = lax.broadcasted_iota(jnp.int32, (8, PAIR), 0)
    lane = lax.broadcasted_iota(jnp.int32, (8, PAIR), 1)
    diag = row == jnp.where(lane >= DH, 1, 0)

    for j in range(3):
        pro_idle(PRO[1 + j])
    assert pos["slab"] >= N_WMA + N_WQ
    wait_filled(wq_v, S_WQ)

    def q_step(p):
        cs = pl.ds(pl.multiple_of(p * PAIR, 128), PAIR)
        qp = jnp.dot(h8, wq_v[:, :, cs].reshape(D, PAIR), preferred_element_type=f32)
        q_s[p] = jnp.where(diag, qp, 0.0)

    pro_compute(NPAIR, q_step)
    assert pos["slab"] >= N_SLAB
    kv_start(k_hbm, 0, 0)
    kv_start(v_hbm, 0, 1)
    pro_idle(PRO[4])
    wait_filled(wmod_v.at[:, :, pl.ds(2 * D, 4 * D)], S_WMB)
    kv_start(k_hbm, 1, 2)
    kv_start(v_hbm, 1, 3)
    pro_compute(10, mod_step(5))
    pro_idle(PRO[5])
    assert pos["piece"] == N_PRO

    scale = DH ** -0.5

    def pair_step(p, acc):
        ks = 2 * lax.rem(p, AHEAD)
        vs = ks + 1
        cur = lax.rem(p, 2)

        wait_filled(kv_ref(ks), S_KV + ks)
        q2 = q_s[p].astype(bf16)
        ch = W // T_QK
        parts = []
        for k in range(T_QK):
            loop_piece(p, k)
            parts.append(jnp.dot(q2, big[ks, :, k * ch:(k + 1) * ch], preferred_element_type=f32))
        s = jnp.concatenate(parts, axis=1) * scale
        e = jnp.exp(s - jnp.max(s, axis=-1, keepdims=True))
        l = jnp.sum(e, axis=-1, keepdims=True)
        e16 = e.astype(bf16)

        @pl.when(p + AHEAD < NPAIR)
        def _():
            kv_start(k_hbm, p + AHEAD, ks)

        ticks(N1, lambda i: loop_piece(p, T_QK + i), PACE)

        wait_filled(wo_ref(cur), S_WO + cur)
        wait_filled(kv_ref(vs), S_KV + vs)
        ch = W // T_PV
        o2 = jnp.zeros((8, PAIR), f32)
        for k in range(T_PV):
            loop_piece(p, T_QK + N1 + k)
            cs = slice(k * ch, (k + 1) * ch)
            o2 = o2 + lax.dot_general(e16[:, cs], big[vs, :, cs], (((1,), (1,)), ((), ())),
                                      preferred_element_type=f32)
        o2 = jnp.where(diag, o2 / l, 0.0).astype(bf16)
        for k in range(PAIR // 128):
            if 1 <= k <= T_WO:
                loop_piece(p, T_QK + N1 + T_PV + k - 1)
            rs = slice(k * 128, (k + 1) * 128)
            acc = acc + jnp.dot(o2[:, rs], big[cur, rs, W:W + D], preferred_element_type=f32)

        @pl.when(p + AHEAD < NPAIR)
        def _():
            kv_start(v_hbm, p + AHEAD, vs)

        @pl.when(p + AHEAD == NPAIR - 1)
        def _():
            w1_cp.start(priority=1)
            for j in range(len(W2_PARTS)):
                w2_cp(j).start(priority=1)

        ticks(jnp.where(p + 1 < NPAIR, N2, 0), lambda i: loop_piece(p, PPP - N2 + i), PACE)
        return acc

    acc = lax.fori_loop(0, NPAIR, pair_step, jnp.zeros((8, D), f32))
    attn = jnp.sum(acc, axis=0, keepdims=True)
    ga, sb, cb, gb = (mod_s[:, i * D:(i + 1) * D] for i in range(2, 6))
    x1 = x32 + ga * attn

    h2 = (_layernorm(x1) * (1.0 + cb) + sb).astype(bf16)
    b1_cp.wait()
    b1 = b1_v[...].astype(f32)
    b1row = jnp.concatenate([b1[j:j + 1, :] for j in range(F // 128)], axis=1)
    wait_filled(w1_v.at[pl.ds(0, W1_ROWS), :], S_W1P)
    w1_cp.wait()
    u = jnp.dot(h2, w1_v[...], preferred_element_type=f32) + b1row
    sp = jnp.log1p(jnp.exp(-jnp.abs(u))) + jnp.maximum(u, 0.0)
    act = (u * jnp.tanh(sp)).astype(bf16)
    wait_filled(w2_ref(0).at[pl.ds(0, W2_ROWS), :], S_W2P)
    y = jnp.zeros((8, D), f32)
    for j, (g, r0, r1) in enumerate(W2_PARTS):
        w2_cp(j).wait()
        r0 = 0 if j == 0 else r0
        y = y + jnp.dot(act[:, g * PAIR + r0:g * PAIR + r1], big[g, r0:r1, W + D:W + 2 * D],
                        preferred_element_type=f32)
    out_v[...] = (x1 + gb * y)[0:1, :].astype(bf16)
    out_cp = copy(out_v, out_hbm, S_OUT)
    out_cp.start()
    out_cp.wait()


@jax.jit
def pallas_adaLN_cond__sliding_block_cached__dense_activation_mish__decode_kernel(
    A_x: jax.Array,
    A_k_cache: jax.Array,
    A_v_cache: jax.Array,
    A_wq: jax.Array,
    A_wo: jax.Array,
    B_x: jax.Array,
    B_w1: jax.Array,
    B_b1: jax.Array,
    B_w2: jax.Array,
    c: jax.Array,
    w_mod: jax.Array,
):
    del B_x
    SK = A_k_cache.shape[2]
    W = min(4096, max(256, SK // 4))
    assert W == sum(KV_COLS)
    kt = jnp.swapaxes(A_k_cache, 2, 3).reshape(H * DH, SK)
    vt = jnp.swapaxes(A_v_cache, 2, 3).reshape(H * DH, SK)
    any_spec = pl.BlockSpec(memory_space=pl.ANY)
    out = pl.pallas_call(
        functools.partial(_kernel, W=W, SK=SK),
        out_shape=jax.ShapeDtypeStruct((1, D), bf16),
        in_specs=[any_spec] * 10,
        out_specs=any_spec,
        scratch_shapes=[
            pltpu.VMEM((1, D), bf16),
            pltpu.VMEM((1, D), bf16),
            pltpu.VMEM((F // 128, 128), bf16),
            pltpu.VMEM((G, GR, 6 * D), bf16),
            pltpu.VMEM((G, GR, H * DH), bf16),
            pltpu.VMEM((NBUF, PAIR, W + 2 * D), bf16),
            pltpu.VMEM((D, F), bf16),
            pltpu.VMEM((NPAIR, 8, PAIR), f32),
            pltpu.VMEM((8, 6 * D), f32),
            pltpu.VMEM((1, D), bf16),
            pltpu.VMEM((8, 128), f32),
            pltpu.SemaphoreType.DMA((NSEM,)),
        ],
        compiler_params=pltpu.CompilerParams(
            vmem_limit_bytes=64 * 1024 * 1024,
            disable_bounds_checks=True,
            disable_semaphore_checks=True,
        ),
    )(A_x.reshape(1, D), c, B_b1.reshape(F // 128, 128), w_mod.reshape(G, GR, 6 * D),
      A_wq.reshape(G, GR, H * DH), kt, vt, A_wo.reshape(NPAIR, PAIR, D), B_w1,
      B_w2.reshape(F // PAIR, PAIR, D))
    return out.reshape(1, 1, D)
```

```python
import functools

import jax
import jax.numpy as jnp
from jax import lax
import jax.experimental.pallas as pl
import jax.experimental.pallas.tpu as pltpu

D = 640
H = 32
DH = 192
F = 1536
PAIR = 2 * DH
NPAIR = H // 2
AHEAD = 2
NBUF = 2 * AHEAD
EPS = 1e-5

G, GR = 10, 64
NRT = GR // 8
WQ_FORMS = ((0, 0, 1792), (0, 1792, 2048), (0, 3840, 2048), (0, 5888, 256),
            (1, 0, 1920), (1, 1920, 1920), (1, 3840, 2304))
NQF = len(WQ_FORMS)
KV_COLS = (1280, 640, 2176)
N_WMB = 2 * NRT
WQ_UP_FRONT = 2
TA, TB, TM = 6, 4, 4

PPP = 96
T_QK, T_PV, T_WO = 8, 16, 2
N1 = 38
N2 = PPP - T_QK - T_PV - T_WO - N1
PRO = (1, 33, 12, 30)
PACE = 64
PACE_TM = 61
N_PRO = (NQF - WQ_UP_FRONT) * TA + (NRT // 2 - 1) * NQF * TB + sum(PRO) + 5 + NPAIR + 10
W1_PIECES = (N_PRO - PPP) // 4 * 4
W1_ROWS = 2 * W1_PIECES
W2_ROWS = 4 * (T_QK + N1 + T_PV + T_WO)
W2_PARTS = ((0, W2_ROWS, PAIR), (1, 0, PAIR), (2, 0, PAIR), (3, 0, 256), (3, 256, PAIR))

f32 = jnp.float32
bf16 = jnp.bfloat16

S_C, S_X, S_B1, S_WMA, S_WMB, S_WQ, S_W1, S_W1P, S_W2P, S_OUT = range(10)
S_WO = 10
S_W2 = S_WO + 2
S_KV = S_W2 + len(W2_PARTS)
NSEM = S_KV + NBUF


def _layernorm(x):
    m = jnp.mean(x, axis=-1, keepdims=True)
    xc = x - m
    v = jnp.mean(xc * xc, axis=-1, keepdims=True)
    return xc / jnp.sqrt(v + EPS)


def _kernel(x_hbm, c_hbm, b1_hbm, wmod_hbm, wq_hbm, k_hbm, v_hbm, wo_hbm, w1_hbm, w2_hbm,
            out_hbm,
            x_v, c_v, b1_v, wmod_v, wq_v, big, w1_v, q_s, mod_s, out_v, pace_s, sem,
            *, W, SK):
    col0 = SK - W

    def kv_ref(slot):
        return big.at[slot, :, pl.ds(0, W)]

    def wo_ref(slot):
        return big.at[slot, :, pl.ds(W, D)]

    def w2_ref(g):
        return big.at[g, :, pl.ds(W + D, D)]

    def mult(v, m):
        return v if isinstance(v, int) else pl.multiple_of(v, m)

    def copy(src, dst, s):
        return pltpu.make_async_copy(src, dst, sem.at[s])

    def wait_filled(buf, s):
        copy(buf, buf, s).wait()

    def ticks(n, tick, pace):
        def body(i, v):
            tick(i)
            for k in range(pace):
                v = v * 0.5 if k % 2 == 0 else v + 0.25
            return v
        pace_s[...] = lax.fori_loop(0, n, body, pace_s[...])

    def slab(src, dst, rt, c0, nc, s):
        idx = (slice(None), pl.ds(mult(8 * rt, 8), 8), pl.ds(mult(c0, 128), nc))
        copy(src.at[idx], dst.at[idx], s).start(priority=1)

    def wq_start(rp, form):
        par, c0, nc = WQ_FORMS[form]
        slab(wq_hbm, wq_v, 2 * rp + par, c0, nc, S_WQ)

    def wmb_start(k):
        @pl.when(k < N_WMB)
        def _():
            slab(wmod_hbm, wmod_v, lax.div(k, 2), (1 + lax.rem(k, 2)) * 2 * D, 2 * D, S_WMB)

    def kv_start(src, p, slot):
        rows = pl.ds(mult(p * PAIR, PAIR), PAIR)
        c0 = 0
        for nc in KV_COLS:
            copy(src.at[rows, pl.ds(col0 + c0, nc)], big.at[slot, :, pl.ds(c0, nc)], S_KV + slot).start(priority=1)
            c0 += nc

    w1_rest = pl.ds(W1_ROWS, D - W1_ROWS)
    w1_cp = copy(w1_hbm.at[w1_rest, :], w1_v.at[w1_rest, :], S_W1)

    def w2_cp(j):
        g, r0, r1 = W2_PARTS[j]
        rows = pl.ds(r0, r1 - r0)
        return copy(w2_hbm.at[g, rows, :], w2_ref(g).at[rows, :], S_W2 + j)

    def row_piece(src, dst, j, s):
        parts = (pl.ds(0, PAIR), pl.ds(PAIR, D - PAIR))
        if isinstance(j, int):
            r = pl.ds(j // 2 * 8, 8)
            copy(src.at[r, parts[j % 2]], dst.at[r, parts[j % 2]], s).start()
            return
        r = pl.ds(pl.multiple_of(lax.div(j, 2) * 8, 8), 8)
        for half in range(2):
            @pl.when(lax.rem(j, 2) == half)
            def _():
                copy(src.at[r, parts[half]], dst.at[r, parts[half]], s).start()

    def pro_piece(j):
        @pl.when(j < W1_PIECES)
        def _():
            idx = (pl.ds(pl.multiple_of(lax.div(j, 4) * 8, 8), 8),
                   pl.ds(pl.multiple_of(lax.rem(j, 4) * PAIR, 128), PAIR))
            copy(w1_hbm.at[idx], w1_v.at[idx], S_W1P).start()

        @pl.when(jnp.logical_and(j >= W1_PIECES, j < W1_PIECES + PPP))
        def _():
            row_piece(wo_hbm.at[0], wo_ref(0), j - W1_PIECES, S_WO)

    def loop_piece(p, j):
        @pl.when(p + 1 < NPAIR)
        def _():
            nxt = lax.rem(p + 1, 2)
            row_piece(wo_hbm.at[p + 1], wo_ref(nxt), j, S_WO + nxt)

        @pl.when(p + 1 == NPAIR)
        def _():
            row_piece(w2_hbm.at[0], w2_ref(0), j, S_W2P)

    x_cp = copy(x_hbm, x_v, S_X)
    c_cp = copy(c_hbm, c_v, S_C)
    b1_cp = copy(b1_hbm, b1_v, S_B1)
    slab(wmod_hbm, wmod_v, 0, 0, 2 * D, S_WMA)
    c_cp.start()
    x_cp.start()
    for rt in range(1, NRT):
        slab(wmod_hbm, wmod_v, rt, 0, 2 * D, S_WMA)
    for form in range(WQ_UP_FRONT):
        wq_start(0, form)
    b1_cp.start()
    pace_s[...] = lax.broadcasted_iota(jnp.int32, (8, 128), 1).astype(f32)

    pos = {"piece": 0, "wmb": 0}

    def pro_tick(n, every):
        j0, k0 = pos["piece"], pos["wmb"]
        pos["piece"] += n
        if every:
            pos["wmb"] += -(-n // every)

        def tick(i):
            pro_piece(j0 + i)
            if every:
                @pl.when(lax.rem(i, every) == 0)
                def _():
                    wmb_start(k0 + lax.div(i, every))
        return tick

    def pro_idle(n, every=0):
        ticks(n, pro_tick(n, every), PACE_TM if every else PACE)

    def pro_compute(n, step, every=0):
        tick = pro_tick(n, every)

        def body(i, carry):
            tick(i)
            step(i)
            return carry
        lax.fori_loop(0, n, body, 0)

    for form in range(WQ_UP_FRONT, NQF):
        pro_idle(TA)
        wq_start(0, form)
    pro_idle(PRO[0])
    c_cp.wait()
    x_cp.wait()
    c32 = c_v[...].astype(f32)
    sc8 = jnp.broadcast_to(c32 * jax.nn.sigmoid(c32), (8, D)).astype(bf16)
    x32 = x_v[...].astype(f32)
    xn = _layernorm(x32)

    def mod_step(first):
        def step(i):
            cs = pl.ds(pl.multiple_of((first + i) * 256, 256), 256)
            mod_s[:, cs] = jnp.dot(sc8, wmod_v[:, :, cs].reshape(D, 256), preferred_element_type=f32)
        return step

    wait_filled(wmod_v.at[:, :, pl.ds(0, 2 * D)], S_WMA)
    pro_compute(5, mod_step(0))
    h8 = (xn * (1.0 + mod_s[:, D:2 * D]) + mod_s[:, 0:D]).astype(bf16)

    row = lax.broadcasted_iota(jnp.int32, (8, PAIR), 0)
    lane = lax.broadcasted_iota(jnp.int32, (8, PAIR), 1)
    diag = row == jnp.where(lane >= DH, 1, 0)

    tick_wq = pro_tick((NRT // 2 - 1) * NQF * TB, 0)

    def wq_rows(rp, carry):
        for form in range(NQF):
            wq_start(rp, form)
            ticks(TB, lambda i: tick_wq(((rp - 1) * NQF + form) * TB + i), PACE)
        return carry

    lax.fori_loop(1, NRT // 2, wq_rows, 0)
    pro_idle(PRO[1], TM)
    wait_filled(wq_v, S_WQ)

    def q_step(p):
        cs = pl.ds(pl.multiple_of(p * PAIR, 128), PAIR)
        qp = jnp.dot(h8, wq_v[:, :, cs].reshape(D, PAIR), preferred_element_type=f32)
        q_s[p] = jnp.where(diag, qp, 0.0)

    pro_compute(NPAIR, q_step, 2)
    assert pos["wmb"] >= N_WMB
    kv_start(k_hbm, 0, 0)
    kv_start(v_hbm, 0, 1)
    pro_idle(PRO[2])
    wait_filled(wmod_v.at[:, :, pl.ds(2 * D, 4 * D)], S_WMB)
    kv_start(k_hbm, 1, 2)
    kv_start(v_hbm, 1, 3)
    pro_compute(10, mod_step(5))
    pro_idle(PRO[3])
    assert pos["piece"] == N_PRO

    scale = DH ** -0.5

    def pair_step(p, acc):
        ks = 2 * lax.rem(p, AHEAD)
        vs = ks + 1
        cur = lax.rem(p, 2)

        wait_filled(kv_ref(ks), S_KV + ks)
        q2 = q_s[p].astype(bf16)
        ch = W // T_QK
        parts = []
        for k in range(T_QK):
            loop_piece(p, k)
            parts.append(jnp.dot(q2, big[ks, :, k * ch:(k + 1) * ch], preferred_element_type=f32))
        s = jnp.concatenate(parts, axis=1) * scale
        e = jnp.exp(s - jnp.max(s, axis=-1, keepdims=True))
        l = jnp.sum(e, axis=-1, keepdims=True)
        e16 = e.astype(bf16)

        @pl.when(p + AHEAD < NPAIR)
        def _():
            kv_start(k_hbm, p + AHEAD, ks)

        ticks(N1, lambda i: loop_piece(p, T_QK + i), PACE)

        wait_filled(wo_ref(cur), S_WO + cur)
        wait_filled(kv_ref(vs), S_KV + vs)
        ch = W // T_PV
        o2 = jnp.zeros((8, PAIR), f32)
        for k in range(T_PV):
            loop_piece(p, T_QK + N1 + k)
            cs = slice(k * ch, (k + 1) * ch)
            o2 = o2 + lax.dot_general(e16[:, cs], big[vs, :, cs], (((1,), (1,)), ((), ())),
                                      preferred_element_type=f32)
        o2 = jnp.where(diag, o2 / l, 0.0).astype(bf16)
        for k in range(PAIR // 128):
            if 1 <= k <= T_WO:
                loop_piece(p, T_QK + N1 + T_PV + k - 1)
            rs = slice(k * 128, (k + 1) * 128)
            acc = acc + jnp.dot(o2[:, rs], big[cur, rs, W:W + D], preferred_element_type=f32)

        @pl.when(p + AHEAD < NPAIR)
        def _():
            kv_start(v_hbm, p + AHEAD, vs)

        @pl.when(p + AHEAD == NPAIR - 1)
        def _():
            w1_cp.start(priority=1)
            for j in range(len(W2_PARTS)):
                w2_cp(j).start(priority=1)

        ticks(jnp.where(p + 1 < NPAIR, N2, 0), lambda i: loop_piece(p, PPP - N2 + i), PACE)
        return acc

    acc = lax.fori_loop(0, NPAIR, pair_step, jnp.zeros((8, D), f32))
    attn = jnp.sum(acc, axis=0, keepdims=True)
    ga, sb, cb, gb = (mod_s[:, i * D:(i + 1) * D] for i in range(2, 6))
    x1 = x32 + ga * attn

    h2 = (_layernorm(x1) * (1.0 + cb) + sb).astype(bf16)
    b1_cp.wait()
    b1 = b1_v[...].astype(f32)
    b1row = jnp.concatenate([b1[j:j + 1, :] for j in range(F // 128)], axis=1)
    wait_filled(w1_v.at[pl.ds(0, W1_ROWS), :], S_W1P)
    w1_cp.wait()
    u = jnp.dot(h2, w1_v[...], preferred_element_type=f32) + b1row
    sp = jnp.log1p(jnp.exp(-jnp.abs(u))) + jnp.maximum(u, 0.0)
    act = (u * jnp.tanh(sp)).astype(bf16)
    wait_filled(w2_ref(0).at[pl.ds(0, W2_ROWS), :], S_W2P)
    y = jnp.zeros((8, D), f32)
    for j, (g, r0, r1) in enumerate(W2_PARTS):
        w2_cp(j).wait()
        r0 = 0 if j == 0 else r0
        y = y + jnp.dot(act[:, g * PAIR + r0:g * PAIR + r1], big[g, r0:r1, W + D:W + 2 * D],
                        preferred_element_type=f32)
    out_v[...] = (x1 + gb * y)[0:1, :].astype(bf16)
    out_cp = copy(out_v, out_hbm, S_OUT)
    out_cp.start()
    out_cp.wait()


@jax.jit
def pallas_adaLN_cond__sliding_block_cached__dense_activation_mish__decode_kernel(
    A_x: jax.Array,
    A_k_cache: jax.Array,
    A_v_cache: jax.Array,
    A_wq: jax.Array,
    A_wo: jax.Array,
    B_x: jax.Array,
    B_w1: jax.Array,
    B_b1: jax.Array,
    B_w2: jax.Array,
    c: jax.Array,
    w_mod: jax.Array,
):
    del B_x
    SK = A_k_cache.shape[2]
    W = min(4096, max(256, SK // 4))
    assert W == sum(KV_COLS)
    kt = jnp.swapaxes(A_k_cache, 2, 3).reshape(H * DH, SK)
    vt = jnp.swapaxes(A_v_cache, 2, 3).reshape(H * DH, SK)
    any_spec = pl.BlockSpec(memory_space=pl.ANY)
    out = pl.pallas_call(
        functools.partial(_kernel, W=W, SK=SK),
        out_shape=jax.ShapeDtypeStruct((1, D), bf16),
        in_specs=[any_spec] * 10,
        out_specs=any_spec,
        scratch_shapes=[
            pltpu.VMEM((1, D), bf16),
            pltpu.VMEM((1, D), bf16),
            pltpu.VMEM((F // 128, 128), bf16),
            pltpu.VMEM((G, GR, 6 * D), bf16),
            pltpu.VMEM((G, GR, H * DH), bf16),
            pltpu.VMEM((NBUF, PAIR, W + 2 * D), bf16),
            pltpu.VMEM((D, F), bf16),
            pltpu.VMEM((NPAIR, 8, PAIR), f32),
            pltpu.VMEM((8, 6 * D), f32),
            pltpu.VMEM((1, D), bf16),
            pltpu.VMEM((8, 128), f32),
            pltpu.SemaphoreType.DMA((NSEM,)),
        ],
        compiler_params=pltpu.CompilerParams(
            vmem_limit_bytes=64 * 1024 * 1024,
            disable_bounds_checks=True,
            disable_semaphore_checks=True,
        ),
    )(A_x.reshape(1, D), c, B_b1.reshape(F // 128, 128), w_mod.reshape(G, GR, 6 * D),
      A_wq.reshape(G, GR, H * DH), kt, vt, A_wo.reshape(NPAIR, PAIR, D), B_w1,
      B_w2.reshape(F // PAIR, PAIR, D))
    return out.reshape(1, 1, D)
```

```python
import functools

import jax
import jax.numpy as jnp
from jax import lax
import jax.experimental.pallas as pl
import jax.experimental.pallas.tpu as pltpu

D = 640
H = 32
DH = 192
F = 1536
PAIR = 2 * DH
NPAIR = H // 2
AHEAD = 2
NBUF = 2 * AHEAD
EPS = 1e-5

G, GR = 10, 64
NRT = GR // 8
WQ_FORMS = ((0, 0, 1792), (0, 1792, 2048), (0, 3840, 2048), (0, 5888, 256),
            (1, 0, 1920), (1, 1920, 1920), (1, 3840, 2304))
NQF = len(WQ_FORMS)
KV_COLS = (1280, 640, 2176)
N_WMB = 2 * NRT
WQ_UP_FRONT = 2
TA, TB, TM = 6, 4, 4

PPP = 96
T_QK, T_PV, T_WO = 8, 16, 2
N1 = 38
N2 = PPP - T_QK - T_PV - T_WO - N1
PRO = (1, 33, 12, 30)
PACE = 64
PACE_TM = 61
N_PRO = (NQF - WQ_UP_FRONT) * TA + (NRT // 2 - 1) * NQF * TB + sum(PRO) + 5 + NPAIR + 10
W1_PIECES = (N_PRO - PPP) // 4 * 4
W1_ROWS = 2 * W1_PIECES
W2_ROWS = 4 * (T_QK + N1 + T_PV + T_WO)
W2_PARTS = ((0, W2_ROWS, PAIR), (1, 0, PAIR), (2, 0, PAIR), (3, 0, 256), (3, 256, 352), (3, 352, PAIR))
N_VPU = 2

f32 = jnp.float32
bf16 = jnp.bfloat16

S_C, S_X, S_B1, S_WMA, S_WMB, S_WQ, S_W1, S_W1P, S_W2P, S_OUT = range(10)
S_WO = 10
S_W2 = S_WO + 2
S_KV = S_W2 + len(W2_PARTS)
NSEM = S_KV + NBUF


def _layernorm(x):
    m = jnp.mean(x, axis=-1, keepdims=True)
    xc = x - m
    v = jnp.mean(xc * xc, axis=-1, keepdims=True)
    return xc / jnp.sqrt(v + EPS)


def _kernel(x_hbm, c_hbm, b1_hbm, wmod_hbm, wq_hbm, k_hbm, v_hbm, wo_hbm, w1_hbm, w2_hbm,
            out_hbm,
            x_v, c_v, b1_v, wmod_v, wq_v, big, w1_v, q_s, mod_s, out_v, pace_s, coef_s, fin_s, sem,
            *, W, SK):
    col0 = SK - W

    def kv_ref(slot):
        return big.at[slot, :, pl.ds(0, W)]

    def wo_ref(slot):
        return big.at[slot, :, pl.ds(W, D)]

    def w2_ref(g):
        return big.at[g, :, pl.ds(W + D, D)]

    def mult(v, m):
        return v if isinstance(v, int) else pl.multiple_of(v, m)

    def copy(src, dst, s):
        return pltpu.make_async_copy(src, dst, sem.at[s])

    def wait_filled(buf, s):
        copy(buf, buf, s).wait()

    def ticks(n, tick, pace):
        def body(i, v):
            tick(i)
            for k in range(pace):
                v = v * 0.5 if k % 2 == 0 else v + 0.25
            return v
        pace_s[...] = lax.fori_loop(0, n, body, pace_s[...])

    def slab(src, dst, rt, c0, nc, s):
        idx = (slice(None), pl.ds(mult(8 * rt, 8), 8), pl.ds(mult(c0, 128), nc))
        copy(src.at[idx], dst.at[idx], s).start(priority=1)

    def wq_start(rp, form):
        par, c0, nc = WQ_FORMS[form]
        slab(wq_hbm, wq_v, 2 * rp + par, c0, nc, S_WQ)

    def wmb_start(k):
        @pl.when(k < N_WMB)
        def _():
            slab(wmod_hbm, wmod_v, lax.div(k, 2), (1 + lax.rem(k, 2)) * 2 * D, 2 * D, S_WMB)

    def kv_start(src, p, slot):
        rows = pl.ds(mult(p * PAIR, PAIR), PAIR)
        c0 = 0
        for nc in KV_COLS:
            copy(src.at[rows, pl.ds(col0 + c0, nc)], big.at[slot, :, pl.ds(c0, nc)], S_KV + slot).start(priority=1)
            c0 += nc

    w1_rest = pl.ds(W1_ROWS, D - W1_ROWS)
    w1_cp = copy(w1_hbm.at[w1_rest, :], w1_v.at[w1_rest, :], S_W1)

    def w2_cp(j):
        g, r0, r1 = W2_PARTS[j]
        rows = pl.ds(r0, r1 - r0)
        return copy(w2_hbm.at[g, rows, :], w2_ref(g).at[rows, :], S_W2 + j)

    def row_piece(src, dst, j, s):
        parts = (pl.ds(0, PAIR), pl.ds(PAIR, D - PAIR))
        if isinstance(j, int):
            r = pl.ds(j // 2 * 8, 8)
            copy(src.at[r, parts[j % 2]], dst.at[r, parts[j % 2]], s).start()
            return
        r = pl.ds(pl.multiple_of(lax.div(j, 2) * 8, 8), 8)
        for half in range(2):
            @pl.when(lax.rem(j, 2) == half)
            def _():
                copy(src.at[r, parts[half]], dst.at[r, parts[half]], s).start()

    def pro_piece(j):
        @pl.when(j < W1_PIECES)
        def _():
            idx = (pl.ds(pl.multiple_of(lax.div(j, 4) * 8, 8), 8),
                   pl.ds(pl.multiple_of(lax.rem(j, 4) * PAIR, 128), PAIR))
            copy(w1_hbm.at[idx], w1_v.at[idx], S_W1P).start()

        @pl.when(jnp.logical_and(j >= W1_PIECES, j < W1_PIECES + PPP))
        def _():
            row_piece(wo_hbm.at[0], wo_ref(0), j - W1_PIECES, S_WO)

    def loop_piece(p, j):
        @pl.when(p + 1 < NPAIR)
        def _():
            nxt = lax.rem(p + 1, 2)
            row_piece(wo_hbm.at[p + 1], wo_ref(nxt), j, S_WO + nxt)

        @pl.when(p + 1 == NPAIR)
        def _():
            row_piece(w2_hbm.at[0], w2_ref(0), j, S_W2P)

    x_cp = copy(x_hbm, x_v, S_X)
    c_cp = copy(c_hbm, c_v, S_C)
    b1_cp = copy(b1_hbm, b1_v, S_B1)
    slab(wmod_hbm, wmod_v, 0, 0, 2 * D, S_WMA)
    c_cp.start()
    x_cp.start()
    for rt in range(1, NRT):
        slab(wmod_hbm, wmod_v, rt, 0, 2 * D, S_WMA)
    for form in range(WQ_UP_FRONT):
        wq_start(0, form)
    b1_cp.start()
    pace_s[...] = lax.broadcasted_iota(jnp.int32, (8, 128), 1).astype(f32)

    pos = {"piece": 0, "wmb": 0}

    def pro_tick(n, every):
        j0, k0 = pos["piece"], pos["wmb"]
        pos["piece"] += n
        if every:
            pos["wmb"] += -(-n // every)

        def tick(i):
            pro_piece(j0 + i)
            if every:
                @pl.when(lax.rem(i, every) == 0)
                def _():
                    wmb_start(k0 + lax.div(i, every))
        return tick

    def pro_idle(n, every=0):
        ticks(n, pro_tick(n, every), PACE_TM if every else PACE)

    def pro_compute(n, step, every=0):
        tick = pro_tick(n, every)

        def body(i, carry):
            tick(i)
            step(i)
            return carry
        lax.fori_loop(0, n, body, 0)

    for form in range(WQ_UP_FRONT, NQF):
        pro_idle(TA)
        wq_start(0, form)
    pro_idle(PRO[0])
    c_cp.wait()
    x_cp.wait()
    c32 = c_v[...].astype(f32)
    sc8 = jnp.broadcast_to(c32 * jax.nn.sigmoid(c32), (8, D)).astype(bf16)
    x32 = x_v[...].astype(f32)
    xn = _layernorm(x32)

    def mod_step(first):
        def step(i):
            cs = pl.ds(pl.multiple_of((first + i) * 256, 256), 256)
            mod_s[:, cs] = jnp.dot(sc8, wmod_v[:, :, cs].reshape(D, 256), preferred_element_type=f32)
        return step

    wait_filled(wmod_v.at[:, :, pl.ds(0, 2 * D)], S_WMA)
    pro_compute(5, mod_step(0))
    h8 = (xn * (1.0 + mod_s[:, D:2 * D]) + mod_s[:, 0:D]).astype(bf16)

    row = lax.broadcasted_iota(jnp.int32, (8, PAIR), 0)
    lane = lax.broadcasted_iota(jnp.int32, (8, PAIR), 1)
    diag = row == jnp.where(lane >= DH, 1, 0)

    tick_wq = pro_tick((NRT // 2 - 1) * NQF * TB, 0)

    def wq_rows(rp, carry):
        for form in range(NQF):
            wq_start(rp, form)
            ticks(TB, lambda i: tick_wq(((rp - 1) * NQF + form) * TB + i), PACE)
        return carry

    lax.fori_loop(1, NRT // 2, wq_rows, 0)
    pro_idle(PRO[1], TM)
    wait_filled(wq_v, S_WQ)

    def q_step(p):
        cs = pl.ds(pl.multiple_of(p * PAIR, 128), PAIR)
        qp = jnp.dot(h8, wq_v[:, :, cs].reshape(D, PAIR), preferred_element_type=f32)
        q_s[p] = jnp.where(diag, qp, 0.0)

    pro_compute(NPAIR, q_step, 2)
    assert pos["wmb"] >= N_WMB
    kv_start(k_hbm, 0, 0)
    kv_start(v_hbm, 0, 1)
    pro_idle(PRO[2])
    wait_filled(wmod_v.at[:, :, pl.ds(2 * D, 4 * D)], S_WMB)
    kv_start(k_hbm, 1, 2)
    kv_start(v_hbm, 1, 3)
    pro_compute(10, mod_step(5))
    pro_idle(PRO[3])
    assert pos["piece"] == N_PRO

    scale = DH ** -0.5

    def pair_step(p, acc):
        ks = 2 * lax.rem(p, AHEAD)
        vs = ks + 1
        cur = lax.rem(p, 2)

        wait_filled(kv_ref(ks), S_KV + ks)
        q2 = q_s[p].astype(bf16)
        ch = W // T_QK
        parts = []
        for k in range(T_QK):
            loop_piece(p, k)
            parts.append(jnp.dot(q2, big[ks, :, k * ch:(k + 1) * ch], preferred_element_type=f32))
        s = jnp.concatenate(parts, axis=1) * scale
        e = jnp.exp(s - jnp.max(s, axis=-1, keepdims=True))
        l = jnp.sum(e, axis=-1, keepdims=True)
        e16 = e.astype(bf16)

        @pl.when(p + AHEAD < NPAIR)
        def _():
            kv_start(k_hbm, p + AHEAD, ks)

        ticks(N1, lambda i: loop_piece(p, T_QK + i), PACE)

        wait_filled(wo_ref(cur), S_WO + cur)
        wait_filled(kv_ref(vs), S_KV + vs)
        ch = W // T_PV
        o2 = jnp.zeros((8, PAIR), f32)
        for k in range(T_PV):
            loop_piece(p, T_QK + N1 + k)
            cs = slice(k * ch, (k + 1) * ch)
            o2 = o2 + lax.dot_general(e16[:, cs], big[vs, :, cs], (((1,), (1,)), ((), ())),
                                      preferred_element_type=f32)
        o2 = jnp.where(diag, o2 / l, 0.0).astype(bf16)
        for k in range(PAIR // 128):
            if 1 <= k <= T_WO:
                loop_piece(p, T_QK + N1 + T_PV + k - 1)
            rs = slice(k * 128, (k + 1) * 128)
            acc = acc + jnp.dot(o2[:, rs], big[cur, rs, W:W + D], preferred_element_type=f32)

        @pl.when(p + AHEAD < NPAIR)
        def _():
            kv_start(v_hbm, p + AHEAD, vs)

        @pl.when(p + AHEAD == NPAIR - 1)
        def _():
            w1_cp.start(priority=1)
            for j in range(len(W2_PARTS)):
                w2_cp(j).start(priority=1)

        ticks(jnp.where(p + 1 < NPAIR, N2, 0), lambda i: loop_piece(p, PPP - N2 + i), PACE)
        return acc

    acc = lax.fori_loop(0, NPAIR, pair_step, jnp.zeros((8, D), f32))
    attn = jnp.sum(acc, axis=0, keepdims=True)
    ga, sb, cb, gb = (mod_s[:, i * D:(i + 1) * D] for i in range(2, 6))
    x1 = x32 + ga * attn

    h2 = (_layernorm(x1) * (1.0 + cb) + sb).astype(bf16)
    b1_cp.wait()
    b1 = b1_v[...].astype(f32)
    b1row = jnp.concatenate([b1[j:j + 1, :] for j in range(F // 128)], axis=1)
    wait_filled(w1_v.at[pl.ds(0, W1_ROWS), :], S_W1P)
    w1_cp.wait()
    u = jnp.dot(h2, w1_v[...], preferred_element_type=f32) + b1row
    sp = jnp.log1p(jnp.exp(-jnp.abs(u))) + jnp.maximum(u, 0.0)
    act = (u * jnp.tanh(sp)).astype(bf16)
    wait_filled(w2_ref(0).at[pl.ds(0, W2_ROWS), :], S_W2P)
    n_mxu = len(W2_PARTS) - N_VPU
    y = jnp.zeros((8, D), f32)
    for j, (g, r0, r1) in enumerate(W2_PARTS[:n_mxu]):
        if j == 2:
            coef_s[...] = jnp.broadcast_to(act[:, F - 128:F].astype(f32).T[:, 0:1], (128, 128))
        w2_cp(j).wait()
        r0 = 0 if j == 0 else r0
        y = y + jnp.dot(act[:, g * PAIR + r0:g * PAIR + r1], big[g, r0:r1, W + D:W + 2 * D],
                        preferred_element_type=f32)
    fin_s[0:8, :] = x1 + gb * y
    fin_s[8:16, :] = gb
    rest = None
    for j, (g, r0, r1) in enumerate(W2_PARTS[n_mxu:], n_mxu):
        w2_cp(j).wait()
        for r in range(r0, r1, 8):
            cf = coef_s[r - (PAIR - 128):r - (PAIR - 128) + 8, :]
            term = big[g, r:r + 8, W + D:W + 2 * D].astype(f32) * jnp.concatenate([cf] * (D // 128), axis=1)
            rest = term if rest is None else rest + term
    res = fin_s[0:8, :] + fin_s[8:16, :] * jnp.sum(rest, axis=0, keepdims=True)
    out_v[...] = res[0:1, :].astype(bf16)
    out_cp = copy(out_v, out_hbm, S_OUT)
    out_cp.start()
    out_cp.wait()


@jax.jit
def pallas_adaLN_cond__sliding_block_cached__dense_activation_mish__decode_kernel(
    A_x: jax.Array,
    A_k_cache: jax.Array,
    A_v_cache: jax.Array,
    A_wq: jax.Array,
    A_wo: jax.Array,
    B_x: jax.Array,
    B_w1: jax.Array,
    B_b1: jax.Array,
    B_w2: jax.Array,
    c: jax.Array,
    w_mod: jax.Array,
):
    del B_x
    SK = A_k_cache.shape[2]
    W = min(4096, max(256, SK // 4))
    assert W == sum(KV_COLS)
    kt = jnp.swapaxes(A_k_cache, 2, 3).reshape(H * DH, SK)
    vt = jnp.swapaxes(A_v_cache, 2, 3).reshape(H * DH, SK)
    any_spec = pl.BlockSpec(memory_space=pl.ANY)
    out = pl.pallas_call(
        functools.partial(_kernel, W=W, SK=SK),
        out_shape=jax.ShapeDtypeStruct((1, D), bf16),
        in_specs=[any_spec] * 10,
        out_specs=any_spec,
        scratch_shapes=[
            pltpu.VMEM((1, D), bf16),
            pltpu.VMEM((1, D), bf16),
            pltpu.VMEM((F // 128, 128), bf16),
            pltpu.VMEM((G, GR, 6 * D), bf16),
            pltpu.VMEM((G, GR, H * DH), bf16),
            pltpu.VMEM((NBUF, PAIR, W + 2 * D), bf16),
            pltpu.VMEM((D, F), bf16),
            pltpu.VMEM((NPAIR, 8, PAIR), f32),
            pltpu.VMEM((8, 6 * D), f32),
            pltpu.VMEM((1, D), bf16),
            pltpu.VMEM((8, 128), f32),
            pltpu.VMEM((128, 128), f32),
            pltpu.VMEM((16, D), f32),
            pltpu.SemaphoreType.DMA((NSEM,)),
        ],
        compiler_params=pltpu.CompilerParams(
            vmem_limit_bytes=64 * 1024 * 1024,
            disable_bounds_checks=True,
            disable_semaphore_checks=True,
        ),
    )(A_x.reshape(1, D), c, B_b1.reshape(F // 128, 128), w_mod.reshape(G, GR, 6 * D),
      A_wq.reshape(G, GR, H * DH), kt, vt, A_wo.reshape(NPAIR, PAIR, D), B_w1,
      B_w2.reshape(F // PAIR, PAIR, D))
    return out.reshape(1, 1, D)
```

```python
import functools

import jax
import jax.numpy as jnp
from jax import lax
import jax.experimental.pallas as pl
import jax.experimental.pallas.tpu as pltpu

D = 640
H = 32
DH = 192
F = 1536
PAIR = 2 * DH
NPAIR = H // 2
AHEAD = 2
NBUF = 2 * AHEAD
EPS = 1e-5

G, GR = 10, 64
NRT = GR // 8
WQ_FORMS = ((0, 0, 1792), (0, 1792, 2048), (0, 3840, 2048), (0, 5888, 256),
            (1, 0, 1920), (1, 1920, 1920), (1, 3840, 2304))
NQF = len(WQ_FORMS)
KV_COLS = (1280, 640, 2176)
N_WMB = 2 * NRT
WQ_UP_FRONT = 2
TA, TB, TM = 6, 4, 4

PPP = 96
T_QK, T_PV, T_WO = 8, 16, 2
N1 = 36
N2 = PPP - T_QK - T_PV - T_WO - N1
PRO = (1, 33, 12, 34)
PACE = 64
PACE_TM = 61
N_PRO = (NQF - WQ_UP_FRONT) * TA + (NRT // 2 - 1) * NQF * TB + sum(PRO) + 5 + NPAIR + 10
W1_PIECES = (N_PRO - PPP) // 4 * 4
W1_ROWS = 2 * W1_PIECES
W2_ROWS = 4 * (T_QK + N1 + T_PV + T_WO)
W2_PARTS = ((0, W2_ROWS, PAIR), (1, 0, PAIR), (2, 0, PAIR), (3, 0, 256), (3, 256, 352), (3, 352, PAIR))
N_VPU = 2

f32 = jnp.float32
bf16 = jnp.bfloat16

S_C, S_X, S_B1, S_WMA, S_WMB, S_WQ, S_W1, S_W1P, S_W2P, S_OUT = range(10)
S_WO = 10
S_W2 = S_WO + 2
S_KV = S_W2 + len(W2_PARTS)
NSEM = S_KV + NBUF


def _layernorm(x):
    m = jnp.mean(x, axis=-1, keepdims=True)
    xc = x - m
    v = jnp.mean(xc * xc, axis=-1, keepdims=True)
    return xc / jnp.sqrt(v + EPS)


def _kernel(x_hbm, c_hbm, b1_hbm, wmod_hbm, wq_hbm, k_hbm, v_hbm, wo_hbm, w1_hbm, w2_hbm,
            out_hbm,
            x_v, c_v, b1_v, wmod_v, wq_v, big, w1_v, q_s, mod_s, out_v, pace_s, coef_s, fin_s, sem,
            *, W, SK):
    col0 = SK - W

    def kv_ref(slot):
        return big.at[slot, :, pl.ds(0, W)]

    def wo_ref(slot):
        return big.at[slot, :, pl.ds(W, D)]

    def w2_ref(g):
        return big.at[g, :, pl.ds(W + D, D)]

    def mult(v, m):
        return v if isinstance(v, int) else pl.multiple_of(v, m)

    def copy(src, dst, s):
        return pltpu.make_async_copy(src, dst, sem.at[s])

    def wait_filled(buf, s):
        copy(buf, buf, s).wait()

    def ticks(n, tick, pace):
        def body(i, v):
            tick(i)
            for k in range(pace):
                v = v * 0.5 if k % 2 == 0 else v + 0.25
            return v
        pace_s[...] = lax.fori_loop(0, n, body, pace_s[...])

    def slab(src, dst, rt, c0, nc, s):
        idx = (slice(None), pl.ds(mult(8 * rt, 8), 8), pl.ds(mult(c0, 128), nc))
        copy(src.at[idx], dst.at[idx], s).start(priority=1)

    def wq_start(rp, form):
        par, c0, nc = WQ_FORMS[form]
        slab(wq_hbm, wq_v, 2 * rp + par, c0, nc, S_WQ)

    def wmb_start(k):
        @pl.when(k < N_WMB)
        def _():
            slab(wmod_hbm, wmod_v, lax.div(k, 2), (1 + lax.rem(k, 2)) * 2 * D, 2 * D, S_WMB)

    def kv_start(src, p, slot):
        rows = pl.ds(mult(p * PAIR, PAIR), PAIR)
        c0 = 0
        for nc in KV_COLS:
            copy(src.at[rows, pl.ds(col0 + c0, nc)], big.at[slot, :, pl.ds(c0, nc)], S_KV + slot).start(priority=1)
            c0 += nc

    w1_rest = pl.ds(W1_ROWS, D - W1_ROWS)
    w1_cp = copy(w1_hbm.at[w1_rest, :], w1_v.at[w1_rest, :], S_W1)

    def w2_cp(j):
        g, r0, r1 = W2_PARTS[j]
        rows = pl.ds(r0, r1 - r0)
        return copy(w2_hbm.at[g, rows, :], w2_ref(g).at[rows, :], S_W2 + j)

    def row_piece(src, dst, j, s):
        parts = (pl.ds(0, PAIR), pl.ds(PAIR, D - PAIR))
        if isinstance(j, int):
            r = pl.ds(j // 2 * 8, 8)
            copy(src.at[r, parts[j % 2]], dst.at[r, parts[j % 2]], s).start()
            return
        r = pl.ds(pl.multiple_of(lax.div(j, 2) * 8, 8), 8)
        for half in range(2):
            @pl.when(lax.rem(j, 2) == half)
            def _():
                copy(src.at[r, parts[half]], dst.at[r, parts[half]], s).start()

    def pro_piece(j):
        @pl.when(j < W1_PIECES)
        def _():
            idx = (pl.ds(pl.multiple_of(lax.div(j, 4) * 8, 8), 8),
                   pl.ds(pl.multiple_of(lax.rem(j, 4) * PAIR, 128), PAIR))
            copy(w1_hbm.at[idx], w1_v.at[idx], S_W1P).start()

        @pl.when(jnp.logical_and(j >= W1_PIECES, j < W1_PIECES + PPP))
        def _():
            row_piece(wo_hbm.at[0], wo_ref(0), j - W1_PIECES, S_WO)

    def wo_piece(p, j):
        nxt = lax.rem(p + 1, 2)
        row_piece(wo_hbm.at[p + 1], wo_ref(nxt), j, S_WO + nxt)

    def loop_piece(p, j):
        @pl.when(p + 1 < NPAIR)
        def _():
            wo_piece(p, j)

        @pl.when(p + 1 == NPAIR)
        def _():
            row_piece(w2_hbm.at[0], w2_ref(0), j, S_W2P)

    x_cp = copy(x_hbm, x_v, S_X)
    c_cp = copy(c_hbm, c_v, S_C)
    b1_cp = copy(b1_hbm, b1_v, S_B1)
    slab(wmod_hbm, wmod_v, 0, 0, 2 * D, S_WMA)
    c_cp.start()
    x_cp.start()
    for rt in range(1, NRT):
        slab(wmod_hbm, wmod_v, rt, 0, 2 * D, S_WMA)
    for form in range(WQ_UP_FRONT):
        wq_start(0, form)
    b1_cp.start()
    pace_s[...] = lax.broadcasted_iota(jnp.int32, (8, 128), 1).astype(f32)

    pos = {"piece": 0, "wmb": 0}

    def pro_tick(n, every):
        j0, k0 = pos["piece"], pos["wmb"]
        pos["piece"] += n
        if every:
            pos["wmb"] += -(-n // every)

        def tick(i):
            pro_piece(j0 + i)
            if every:
                @pl.when(lax.rem(i, every) == 0)
                def _():
                    wmb_start(k0 + lax.div(i, every))
        return tick

    def pro_idle(n, every=0):
        ticks(n, pro_tick(n, every), PACE_TM if every else PACE)

    def pro_compute(n, step, every=0):
        tick = pro_tick(n, every)

        def body(i, carry):
            tick(i)
            step(i)
            return carry
        lax.fori_loop(0, n, body, 0)

    for form in range(WQ_UP_FRONT, NQF):
        pro_idle(TA)
        wq_start(0, form)
    pro_idle(PRO[0])
    c_cp.wait()
    x_cp.wait()
    c32 = c_v[...].astype(f32)
    sc8 = jnp.broadcast_to(c32 * jax.nn.sigmoid(c32), (8, D)).astype(bf16)
    x32 = x_v[...].astype(f32)
    xn = _layernorm(x32)

    def mod_step(first):
        def step(i):
            cs = pl.ds(pl.multiple_of((first + i) * 256, 256), 256)
            mod_s[:, cs] = jnp.dot(sc8, wmod_v[:, :, cs].reshape(D, 256), preferred_element_type=f32)
        return step

    wait_filled(wmod_v.at[:, :, pl.ds(0, 2 * D)], S_WMA)
    pro_compute(5, mod_step(0))
    h8 = (xn * (1.0 + mod_s[:, D:2 * D]) + mod_s[:, 0:D]).astype(bf16)

    row = lax.broadcasted_iota(jnp.int32, (8, PAIR), 0)
    lane = lax.broadcasted_iota(jnp.int32, (8, PAIR), 1)
    diag = row == jnp.where(lane >= DH, 1, 0)

    tick_wq = pro_tick((NRT // 2 - 1) * NQF * TB, 0)

    def wq_rows(rp, carry):
        for form in range(NQF):
            wq_start(rp, form)
            ticks(TB, lambda i: tick_wq(((rp - 1) * NQF + form) * TB + i), PACE)
        return carry

    lax.fori_loop(1, NRT // 2, wq_rows, 0)
    pro_idle(PRO[1], TM)
    wait_filled(wq_v, S_WQ)

    def q_step(p):
        cs = pl.ds(pl.multiple_of(p * PAIR, 128), PAIR)
        qp = jnp.dot(h8, wq_v[:, :, cs].reshape(D, PAIR), preferred_element_type=f32)
        q_s[p] = jnp.where(diag, qp, 0.0)

    pro_compute(NPAIR, q_step, 2)
    assert pos["wmb"] >= N_WMB
    kv_start(k_hbm, 0, 0)
    kv_start(v_hbm, 0, 1)
    pro_idle(PRO[2])
    wait_filled(wmod_v.at[:, :, pl.ds(2 * D, 4 * D)], S_WMB)
    kv_start(k_hbm, 1, 2)
    kv_start(v_hbm, 1, 3)
    pro_compute(10, mod_step(5))
    pro_idle(PRO[3])
    assert pos["piece"] == N_PRO

    scale = DH ** -0.5

    def pair_step(p, acc):
        ks = 2 * lax.rem(p, AHEAD)
        vs = ks + 1
        cur = lax.rem(p, 2)

        wait_filled(kv_ref(ks), S_KV + ks)
        q2 = q_s[p].astype(bf16)
        ch = W // T_QK
        parts = []
        for k in range(T_QK):
            loop_piece(p, k)
            parts.append(jnp.dot(q2, big[ks, :, k * ch:(k + 1) * ch], preferred_element_type=f32))
        s = jnp.concatenate(parts, axis=1) * scale
        e = jnp.exp(s - jnp.max(s, axis=-1, keepdims=True))
        l = jnp.sum(e, axis=-1, keepdims=True)
        e16 = e.astype(bf16)

        @pl.when(p + AHEAD < NPAIR)
        def _():
            kv_start(k_hbm, p + AHEAD, ks)

        ticks(N1, lambda i: loop_piece(p, T_QK + i), PACE)

        wait_filled(wo_ref(cur), S_WO + cur)
        wait_filled(kv_ref(vs), S_KV + vs)
        ch = W // T_PV
        o2 = jnp.zeros((8, PAIR), f32)
        for k in range(T_PV):
            loop_piece(p, T_QK + N1 + k)
            cs = slice(k * ch, (k + 1) * ch)
            o2 = o2 + lax.dot_general(e16[:, cs], big[vs, :, cs], (((1,), (1,)), ((), ())),
                                      preferred_element_type=f32)
        o2 = jnp.where(diag, o2 / l, 0.0).astype(bf16)
        for k in range(PAIR // 128):
            if 1 <= k <= T_WO:
                loop_piece(p, T_QK + N1 + T_PV + k - 1)
            rs = slice(k * 128, (k + 1) * 128)
            acc = acc + jnp.dot(o2[:, rs], big[cur, rs, W:W + D], preferred_element_type=f32)

        @pl.when(p + AHEAD < NPAIR)
        def _():
            kv_start(v_hbm, p + AHEAD, vs)

        @pl.when(p + AHEAD == NPAIR - 1)
        def _():
            w1_cp.start(priority=1)
            for j in range(len(W2_PARTS)):
                w2_cp(j).start(priority=1)

        @pl.when(p + 1 < NPAIR)
        def _():
            ticks(N2, lambda i: wo_piece(p, PPP - N2 + i), PACE)

        return acc

    acc = lax.fori_loop(0, NPAIR, pair_step, jnp.zeros((8, D), f32))
    attn = jnp.sum(acc, axis=0, keepdims=True)
    ga, sb, cb, gb = (mod_s[:, i * D:(i + 1) * D] for i in range(2, 6))
    x1 = x32 + ga * attn

    h2 = (_layernorm(x1) * (1.0 + cb) + sb).astype(bf16)
    b1_cp.wait()
    b1 = b1_v[...].astype(f32)
    b1row = jnp.concatenate([b1[j:j + 1, :] for j in range(F // 128)], axis=1)
    wait_filled(w1_v.at[pl.ds(0, W1_ROWS), :], S_W1P)
    w1_cp.wait()
    u = jnp.dot(h2, w1_v[...], preferred_element_type=f32) + b1row
    sp = jnp.log1p(jnp.exp(-jnp.abs(u))) + jnp.maximum(u, 0.0)
    act = (u * jnp.tanh(sp)).astype(bf16)
    wait_filled(w2_ref(0).at[pl.ds(0, W2_ROWS), :], S_W2P)
    n_mxu = len(W2_PARTS) - N_VPU
    y = jnp.zeros((8, D), f32)
    for j, (g, r0, r1) in enumerate(W2_PARTS[:n_mxu]):
        if j == 2:
            coef_s[...] = jnp.broadcast_to(act[:, F - 128:F].astype(f32).T[:, 0:1], (128, 128))
        w2_cp(j).wait()
        r0 = 0 if j == 0 else r0
        y = y + jnp.dot(act[:, g * PAIR + r0:g * PAIR + r1], big[g, r0:r1, W + D:W + 2 * D],
                        preferred_element_type=f32)
    fin_s[0:8, :] = x1 + gb * y
    fin_s[8:16, :] = gb
    rest = None
    for j, (g, r0, r1) in enumerate(W2_PARTS[n_mxu:], n_mxu):
        w2_cp(j).wait()
        for r in range(r0, r1, 8):
            cf = coef_s[r - (PAIR - 128):r - (PAIR - 128) + 8, :]
            term = big[g, r:r + 8, W + D:W + 2 * D].astype(f32) * jnp.concatenate([cf] * (D // 128), axis=1)
            rest = term if rest is None else rest + term
    res = fin_s[0:8, :] + fin_s[8:16, :] * jnp.sum(rest, axis=0, keepdims=True)
    out_v[...] = res[0:1, :].astype(bf16)
    out_cp = copy(out_v, out_hbm, S_OUT)
    out_cp.start()
    out_cp.wait()


@jax.jit
def pallas_adaLN_cond__sliding_block_cached__dense_activation_mish__decode_kernel(
    A_x: jax.Array,
    A_k_cache: jax.Array,
    A_v_cache: jax.Array,
    A_wq: jax.Array,
    A_wo: jax.Array,
    B_x: jax.Array,
    B_w1: jax.Array,
    B_b1: jax.Array,
    B_w2: jax.Array,
    c: jax.Array,
    w_mod: jax.Array,
):
    del B_x
    SK = A_k_cache.shape[2]
    W = min(4096, max(256, SK // 4))
    assert W == sum(KV_COLS)
    kt = jnp.swapaxes(A_k_cache, 2, 3).reshape(H * DH, SK)
    vt = jnp.swapaxes(A_v_cache, 2, 3).reshape(H * DH, SK)
    any_spec = pl.BlockSpec(memory_space=pl.ANY)
    out = pl.pallas_call(
        functools.partial(_kernel, W=W, SK=SK),
        out_shape=jax.ShapeDtypeStruct((1, D), bf16),
        in_specs=[any_spec] * 10,
        out_specs=any_spec,
        scratch_shapes=[
            pltpu.VMEM((1, D), bf16),
            pltpu.VMEM((1, D), bf16),
            pltpu.VMEM((F // 128, 128), bf16),
            pltpu.VMEM((G, GR, 6 * D), bf16),
            pltpu.VMEM((G, GR, H * DH), bf16),
            pltpu.VMEM((NBUF, PAIR, W + 2 * D), bf16),
            pltpu.VMEM((D, F), bf16),
            pltpu.VMEM((NPAIR, 8, PAIR), f32),
            pltpu.VMEM((8, 6 * D), f32),
            pltpu.VMEM((1, D), bf16),
            pltpu.VMEM((8, 128), f32),
            pltpu.VMEM((128, 128), f32),
            pltpu.VMEM((16, D), f32),
            pltpu.SemaphoreType.DMA((NSEM,)),
        ],
        compiler_params=pltpu.CompilerParams(
            vmem_limit_bytes=100 * 1024 * 1024,
            disable_bounds_checks=True,
            disable_semaphore_checks=True,
        ),
    )(A_x.reshape(1, D), c, B_b1.reshape(F // 128, 128), w_mod.reshape(G, GR, 6 * D),
      A_wq.reshape(G, GR, H * DH), kt, vt, A_wo.reshape(NPAIR, PAIR, D), B_w1,
      B_w2.reshape(F // PAIR, PAIR, D))
    return out.reshape(1, 1, D)
```
